```python
import jax
import jax.numpy as jnp

def _softmax(x, axis=-1):
    return jax.nn.softmax(x, axis=axis)
def _gelu(x):
    return jax.nn.gelu(x, approximate=True)
def _silu(x):
    return jax.nn.silu(x)
def _sigmoid(x):
    return jax.nn.sigmoid(x)
def _layernorm(x, axis=-1, eps=1e-5):
    m = jnp.mean(x, axis=axis, keepdims=True)
    v = jnp.var(x, axis=axis, keepdims=True)
    return (x - m) / jnp.sqrt(v + eps)
def _scatter_add(tgt, idx, src, axis=0):
    return tgt.at[idx].add(src)
def _segment_sum(src, seg, n):
    return jax.ops.segment_sum(src, seg, n)
class _Rng:
    def __init__(self, key):
        self._k = key
    def _next(self):
        self._k, sub = jax.random.split(self._k)
        return sub
    def normal(self, shape):
        return jax.random.normal(self._next(), shape, dtype=jnp.bfloat16)
    def randint(self, lo, hi, shape):
        return jax.random.randint(self._next(), shape, lo, hi, dtype=jnp.int32)
    def uniform(self, shape, lo=0.0, hi=1.0):
        return jax.random.uniform(self._next(), shape, jnp.bfloat16, lo, hi)
    def permutation(self, n):
        return jax.random.permutation(self._next(), n)


kernel_name = 'interleave_layers__sliding_local_dilated__glu_gated_geglu__prompt'

def setup_inputs():
    _rng = _Rng(jax.random.key(int.from_bytes(__import__("os").urandom(4), "little")))
    _w = (lambda a: (lambda t: t.astype(jnp.bfloat16) if jnp.issubdtype(t.dtype, jnp.floating) else t)(jnp.asarray(a)))
    def _A_setup():
        B, S, D = 1, 2048, 576
        return {
            "x": _w((lambda *s: _rng.normal(s) * 0.05)(B, S, D)),
            "wqkv": _w((lambda *s: _rng.normal(s) * 0.05)(D, 3 * D)),
            "wo": _w((lambda *s: _rng.normal(s) * 0.05)(D, D)),
        }
    _A_in = _A_setup()

    def _B_setup():
        B, S, Dm, Df = 1, 2048, 576, 4608
        return {
            "x": _w((lambda *s: _rng.normal(s) * 0.05)(B, S, Dm)),
            "w_gate": _w((lambda *s: _rng.normal(s) * 0.05)(Dm, Df) * (Dm ** -0.5)),
            "w_up": _w((lambda *s: _rng.normal(s) * 0.05)(Dm, Df) * (Dm ** -0.5)),
            "w_down": _w((lambda *s: _rng.normal(s) * 0.05)(Df, Dm) * (Df ** -0.5)),
        }
    _B_in = _B_setup()

    return {
        "A_x": _A_in["x"],
        "A_wqkv": _A_in["wqkv"],
        "A_wo": _A_in["wo"],
        "B_x": _B_in["x"],
        "B_w_gate": _B_in["w_gate"],
        "B_w_up": _B_in["w_up"],
        "B_w_down": _B_in["w_down"],
    }

def reference(A_x, A_wqkv, A_wo, B_x, B_w_gate, B_w_up, B_w_down):
    def _A_ref(x, wqkv, wo):
        B, S, D = x.shape
        H = 32; Dh = D // H
        W, dil = 8, 2
        qkv = (lambda x, *d: x.transpose(*d))((x @ wqkv).reshape(B, S, 3, H, Dh), 2, 0, 3, 1, 4)
        q, k, v = qkv[0], qkv[1], qkv[2]
        scale = Dh ** -0.5
        pos = jnp.arange(S)
        off = jnp.arange(W) * dil
        idx = pos[:, None] - off[None, :]
        mask = idx >= 0
        idx_c = jnp.where(mask, idx, 0).reshape(-1)
        kg = k[:, :, idx_c, :].reshape(B, H, S, W, Dh)
        vg = v[:, :, idx_c, :].reshape(B, H, S, W, Dh)
        logits = jnp.einsum("bhsd,bhswd->bhsw", q, kg) * scale
        logits = jnp.where(mask[None, None, :, :], logits, -1e9)
        attn = _softmax(logits, axis=-1)
        o = jnp.einsum("bhsw,bhswd->bhsd", attn, vg)
        return (lambda x, *d: x.transpose(*d))(o, 0, 2, 1, 3).reshape(B, S, D) @ wo

    def _B_ref(x, w_gate, w_up, w_down):
        g = jnp.einsum("bsd,df->bsf", x, w_gate)
        u = jnp.einsum("bsd,df->bsf", x, w_up)
        h = _gelu(g) * u
        return jnp.einsum("bsf,fd->bsd", h, w_down)

    x = A_x
    x = x + _A_ref(_layernorm(x, axis=-1), A_wqkv, A_wo)
    x = x + _B_ref(_layernorm(x, axis=-1), B_w_gate, B_w_up, B_w_down)
    x = x + _A_ref(_layernorm(x, axis=-1), A_wqkv, A_wo)
    x = x + _B_ref(_layernorm(x, axis=-1), B_w_gate, B_w_up, B_w_down)
    return x
```

```python
import functools
import numpy as np
import jax
import jax.numpy as jnp
from jax import lax
import jax.experimental.pallas as pl
import jax.experimental.pallas.tpu as pltpu

S, D, F, H, DH = 2048, 576, 4608, 32, 18
NW, DIL = 8, 2
HALO = 16
LOG2E = 1.4426950408889634
NT = (((1,), (1,)), ((), ()))
F32, BF16 = jnp.float32, jnp.bfloat16

def _ln_t(x):
    m = jnp.sum(x, axis=0, keepdims=True) * (1.0 / D)
    xc = x - m
    v = jnp.sum(xc * xc, axis=0, keepdims=True) * (1.0 / D)
    return (xc * lax.rsqrt(v + 1e-5)).astype(BF16)

def _gelu(g):
    c = np.float32(np.sqrt(2 / np.pi))
    inner = g * (c + (c * 0.044715) * (g * g))
    hg = 0.5 * g
    return hg + hg * jnp.tanh(inner)

def make_kernel(TM=512, FC=1152, FS=1152, RT=16, ablate=''):
    NB = S // TM
    NF = F // FC
    NSLOT = 2 * NB + 1
    PR = TM // NF

    def blk_of(a):
        return 2 * (a // 4) + a % 2

    def kernel(x_ref, wqkv_hbm, wo_hbm, wg_hbm, wu_hbm, wd_hbm, o_ref,
               wraw, woraw, t32, wqt, wot, wg, wu, wd, xs, xna, xnf, qs, kb, vb, os_, sems):
        s = pl.program_id(0)
        def cp_qkv(): return pltpu.make_async_copy(wqkv_hbm, wraw, sems.at[0])
        def cp_o(): return pltpu.make_async_copy(wo_hbm, woraw, sems.at[1])
        def cp_g(f): return pltpu.make_async_copy(wg_hbm.at[:, pl.ds(f*FC, FC)], wg.at[f], sems.at[2+3*f])
        def cp_u(f): return pltpu.make_async_copy(wu_hbm.at[:, pl.ds(f*FC, FC)], wu.at[f], sems.at[3+3*f])
        def cp_d(f): return pltpu.make_async_copy(wd_hbm.at[:, pl.ds(f*FC, FC)], wd.at[f], sems.at[4+3*f])

        @pl.when(s == 0)
        def _():
            cp_qkv().start(); cp_o().start()
            for f in range(NF):
                cp_g(f).start(); cp_u(f).start(); cp_d(f).start()
            os_[...] = jnp.zeros(os_.shape, BF16)
            xs[1] = jnp.zeros((D, TM), F32)
            cp_qkv().wait()
            for c in range(5):
                kw = 128 if c < 4 else 64
                for j in range(14):
                    nw = 128 if j < 13 else 64
                    blk = wraw[c*128:c*128+kw, j*128:j*128+nw].astype(F32)
                    if kw < 128: blk = jnp.concatenate([blk, jnp.zeros((128-kw, nw), F32)], axis=0)
                    if nw < 128: blk = jnp.concatenate([blk, jnp.zeros((128, 128-nw), F32)], axis=1)
                    t32[c, j*128:(j+1)*128, :] = blk.T
            wqt[1728:1792, :] = jnp.zeros((64, 640), BF16)
            def dest(p, d):
                if p == 0: return d * 32
                if p == 1: return 576 + (d - 16) * 32 if d >= 16 else 640 + d * 32
                return 1152 + d * 32
            for p in range(3):
                for d in range(DH):
                    for c in range(5):
                        rows = t32[c, pl.ds(p * D + d, H, stride=DH), :]
                        r0 = dest(p, d)
                        wqt[r0:r0+H, c*128:(c+1)*128] = rows.astype(BF16)
            cp_o().wait()
            for c in range(5):
                nw = 128 if c < 4 else 64
                blk = woraw[:, c*128:c*128+nw].astype(F32)
                if nw < 128: blk = jnp.concatenate([blk, jnp.zeros((D, 128-nw), F32)], axis=1)
                t32[c, 0:D, :] = blk
            for c in range(5):
                parts = [t32[c, pl.ds(d, H, stride=DH), :] for d in range(DH)] + [jnp.zeros((64, 128), F32)]
                wp = jnp.concatenate(parts, axis=0)
                res = wp.T.astype(BF16)
                nw = 128 if c < 4 else 64
                wot[c*128:c*128+nw, :] = res[:nw]

        pa = s % 2
        pf = 1 - pa
        la = (s // 2) % 2
        ab = blk_of(s)
        qscale = (DH ** -0.5) * LOG2E

        @pl.when(la == 0)
        def _():
            xs[pa] = x_ref[...].astype(F32)

        xs[pf] += lax.dot_general(wot[:, 0:D], os_[:, 0:D], NT, preferred_element_type=F32)
        xna[:, 0:D] = _ln_t(xs[pa]).T

        @pl.when(s < NSLOT - 1)
        def _():
            for c in range(5):
                kb[la, c, 0:HALO, :] = kb[la, c, TM:TM+HALO, :]
                vb[la, c, 0:HALO, :] = vb[la, c, TM:TM+HALO, :]
            xnf[:, 0:D] = _ln_t(xs[pf]).T
            qkv = lax.dot_general(xna[:, 0:D], wqt[:, 0:D], NT, preferred_element_type=F32)
            lane = lax.broadcasted_iota(jnp.int32, (TM, 128), 1)
            qs[:, 0:512] = qkv[:, 0:512] * qscale
            t4 = qkv[:, 512:640]
            qs[:, 512:640] = jnp.where(lane < 64, t4 * qscale, 0.0)
            for c in range(4):
                kb[la, c, HALO:, :] = qkv[:, 640+c*128:640+(c+1)*128]
            kb[la, 4, HALO:, :] = pltpu.roll(t4, 64, 1)
            for c in range(5):
                vb[la, c, HALO:, :] = qkv[:, 1152+c*128:1152+(c+1)*128]

        @pl.when(s == NSLOT - 1)
        def _():
            xnf[:, 0:D] = _ln_t(xs[pf]).T

        @pl.when(ab == 0)
        def _():
            for c in range(5):
                kb[la, c, 0:HALO, :] = jnp.zeros((HALO, 128), F32)
                vb[la, c, 0:HALO, :] = jnp.broadcast_to(vb[la, c, HALO:HALO+1, :], (HALO, 128))

        def att_tile(r0, masked):
            q = [qs[pl.ds(r0, RT), c*128:(c+1)*128] for c in range(5)]
            lg = []
            for w in range(NW):
                acc = None
                for c in range(5):
                    kk = kb[la, c, pl.ds(r0 + HALO - DIL*w, RT), :]
                    p = q[c] * kk
                    acc = p if acc is None else acc + p
                acc = acc + pltpu.roll(acc, 64, 1)
                acc = acc + pltpu.roll(acc, 32, 1)
                if masked and w > 0:
                    pos = ab * TM + r0 + lax.broadcasted_iota(jnp.int32, (RT, 128), 0)
                    acc = jnp.where(pos >= DIL*w, acc, -1e9 * LOG2E)
                lg.append(acc)
            mx = lg[0]
            for w in range(1, NW): mx = jnp.maximum(mx, lg[w])
            e = [jnp.exp2(a - mx) for a in lg]
            sm = e[0]
            for w in range(1, NW): sm = sm + e[w]
            inv = 1.0 / sm
            for c in range(5):
                acc = None
                for w in range(NW):
                    vv = vb[la, c, pl.ds(r0 + HALO - DIL*w, RT), :]
                    t = e[w] * vv
                    acc = t if acc is None else acc + t
                os_[pl.ds(r0, RT), c*128:(c+1)*128] = (acc * inv).astype(BF16)

        def att_piece(f):
            if 'noatt' in ablate: return
            base = pl.multiple_of(f * PR, PR)
            for r in range(PR // RT):
                att_tile(base + r * RT, masked=(r == 0))

        def ffn_chunk(f):
            xn = xnf[:, 0:D]
            for j in range(FC // FS):
                g = jnp.dot(xn, wg[f, :, j*FS:(j+1)*FS], preferred_element_type=F32)
                u = jnp.dot(xn, wu[f, :, j*FS:(j+1)*FS], preferred_element_type=F32)
                h = (_gelu(g) * u).astype(BF16)
                xs[pf] += lax.dot_general(wd[f, :, j*FS:(j+1)*FS], h, NT, preferred_element_type=F32)

        @pl.when(s == 0)
        def _():
            def body(f, _):
                att_piece(f); return 0
            lax.fori_loop(0, NF, body, 0)

        @pl.when(s > 0)
        def _():
            def body(f, _):
                @pl.when(s == 1)
                def _():
                    for ff in range(NF):
                        @pl.when(f == ff)
                        def _():
                            cp_g(ff).wait(); cp_u(ff).wait(); cp_d(ff).wait()
                ffn_chunk(f)
                att_piece(f)
                return 0
            lax.fori_loop(0, NF, body, 0)

        @pl.when(jnp.logical_and(s > 0, ((s - 1) // 2) % 2 == 1))
        def _():
            o_ref[...] = xs[pf].astype(o_ref.dtype)

    def x_map(s):
        la = (s // 2) % 2
        b = jnp.where(la == 0, blk_of(s), 2 * (s // 4) + 1)
        return (0, jnp.minimum(b, NB - 1))

    def o_map(s):
        fidx = jnp.maximum(s - 1, 0)
        b = 2 * (fidx // 4) + jnp.where(fidx % 4 == 3, 1, 0)
        return (0, b)

    def fn(A_x, A_wqkv, A_wo, B_x, B_w_gate, B_w_up, B_w_down):
        xT = A_x.reshape(S, D).T
        out = pl.pallas_call(
            kernel,
            grid=(NSLOT,),
            in_specs=[pl.BlockSpec((D, TM), x_map)] + [pl.BlockSpec(memory_space=pltpu.HBM)] * 5,
            out_specs=pl.BlockSpec((D, TM), o_map),
            out_shape=jax.ShapeDtypeStruct((D, S), BF16),
            scratch_shapes=[
                pltpu.VMEM((D, 3 * D), BF16), pltpu.VMEM((D, D), BF16),
                pltpu.VMEM((5, 1792, 128), F32),
                pltpu.VMEM((1792, 640), BF16), pltpu.VMEM((D, 640), BF16),
                pltpu.VMEM((NF, D, FC), BF16), pltpu.VMEM((NF, D, FC), BF16), pltpu.VMEM((NF, D, FC), BF16),
                pltpu.VMEM((2, D, TM), F32), pltpu.VMEM((TM, 640), BF16), pltpu.VMEM((TM, 640), BF16),
                pltpu.VMEM((TM, 640), F32),
                pltpu.VMEM((2, 5, TM + HALO, 128), F32), pltpu.VMEM((2, 5, TM + HALO, 128), F32),
                pltpu.VMEM((TM, 640), BF16),
                pltpu.SemaphoreType.DMA((2 + 3 * NF,)),
            ],
            compiler_params=pltpu.CompilerParams(dimension_semantics=("arbitrary",), vmem_limit_bytes=100 * 1024 * 1024),
        )(xT, A_wqkv, A_wo, B_w_gate, B_w_up, B_w_down.T)
        return out.T.reshape(1, S, D)
    return fn


_fn = make_kernel(TM=512, FC=1152, FS=1152)


@jax.jit
def pallas_interleave_layers__sliding_local_dilated__glu_gated_geglu__prompt_kernel(
    A_x: jax.Array,
    A_wqkv: jax.Array,
    A_wo: jax.Array,
    B_x: jax.Array,
    B_w_gate: jax.Array,
    B_w_up: jax.Array,
    B_w_down: jax.Array,
):
    return _fn(A_x, A_wqkv, A_wo, B_x, B_w_gate, B_w_up, B_w_down)
```

```python
import functools
import numpy as np
import jax
import jax.numpy as jnp
from jax import lax
import jax.experimental.pallas as pl
import jax.experimental.pallas.tpu as pltpu

S, D, F, H, DH = 2048, 576, 4608, 32, 18
NW, DIL = 8, 2
HALO = 16
LOG2E = 1.4426950408889634
NT = (((1,), (1,)), ((), ()))
F32, BF16 = jnp.float32, jnp.bfloat16

def _ln_t(x):
    m = jnp.sum(x, axis=0, keepdims=True) * (1.0 / D)
    xc = x - m
    v = jnp.sum(xc * xc, axis=0, keepdims=True) * (1.0 / D)
    return (xc * lax.rsqrt(v + 1e-5)).astype(BF16)

def _gelu(g):
    c = np.float32(np.sqrt(2 / np.pi))
    inner = g * (c + (c * 0.044715) * (g * g))
    hg = 0.5 * g
    return hg + hg * jnp.tanh(inner)

def make_kernel(TM=512, FC=1152, FS=1152, RT=16, RTP=32, LNC=128, ablate=''):
    NB = S // TM
    NF = F // FC
    NSLOT = 2 * NB + 1
    PR = TM // NF

    def blk_of(a):
        return 2 * (a // 4) + a % 2

    def kernel(x_ref, x1_ref, wqkv_hbm, wo_hbm, wg_hbm, wu_hbm, wd_hbm, o_ref,
               wraw, woraw, t32, wqt, wot, wg, wu, wd, xs, xna, xnf, qs, kb, vb, kt, vt, os_, sems):
        s = pl.program_id(0)
        def cp_qkv(): return pltpu.make_async_copy(wqkv_hbm, wraw, sems.at[0])
        def cp_o(): return pltpu.make_async_copy(wo_hbm, woraw, sems.at[1])
        def cp_g(f): return pltpu.make_async_copy(wg_hbm.at[:, pl.ds(f*FC, FC)], wg.at[f], sems.at[2+3*f])
        def cp_u(f): return pltpu.make_async_copy(wu_hbm.at[:, pl.ds(f*FC, FC)], wu.at[f], sems.at[3+3*f])
        def cp_d(f): return pltpu.make_async_copy(wd_hbm.at[:, pl.ds(f*FC, FC)], wd.at[f], sems.at[4+3*f])

        qscale = (DH ** -0.5) * LOG2E

        def prep():
            cp_qkv().start(); cp_o().start()
            if 'latedma' not in ablate:
                for f in range(NF):
                    cp_g(f).start(); cp_u(f).start(); cp_d(f).start()
            cp_qkv().wait()
            if 'latedma' in ablate:
                for f in range(NF):
                    cp_g(f).start(); cp_u(f).start(); cp_d(f).start()
            for c in range(5):
                kw = 128 if c < 4 else 64
                for j in range(14):
                    nw = 128 if j < 13 else 64
                    blk = wraw[c*128:c*128+kw, j*128:j*128+nw].astype(F32)
                    if kw < 128: blk = jnp.concatenate([blk, jnp.zeros((128-kw, nw), F32)], axis=0)
                    if nw < 128: blk = jnp.concatenate([blk, jnp.zeros((128, 128-nw), F32)], axis=1)
                    t32[c, j*128:(j+1)*128, :] = blk.T
            wqt[1728:1792, :] = jnp.zeros((64, 640), BF16)
            def dest(p, d):
                if p == 0: return d * 32
                if p == 1: return 576 + (d - 16) * 32 if d >= 16 else 640 + d * 32
                return 1152 + d * 32
            for p in range(3):
                for d in range(DH):
                    for c in range(5):
                        rows = t32[c, pl.ds(p * D + d, H, stride=DH), :]
                        r0 = dest(p, d)
                        wqt[r0:r0+H, c*128:(c+1)*128] = rows.astype(BF16)

        def prep_wo():
            cp_o().wait()
            for c in range(5):
                nw = 128 if c < 4 else 64
                blk = woraw[:, c*128:c*128+nw].astype(F32)
                if nw < 128: blk = jnp.concatenate([blk, jnp.zeros((D, 128-nw), F32)], axis=1)
                t32[c, 0:D, :] = blk
            for c in range(5):
                parts = [t32[c, pl.ds(d, H, stride=DH), :] for d in range(DH)] + [jnp.zeros((64, 128), F32)]
                wp = jnp.concatenate(parts, axis=0)
                res = wp.T.astype(BF16)
                nw = 128 if c < 4 else 64
                wot[c*128:c*128+nw, :] = res[:nw]

        def ln_to(dst, get):
            for c0 in range(0, TM, LNC):
                dst[c0:c0+LNC, 0:D] = _ln_t(get(c0)).T

        def ln_a(pa, xin, use_in):
            def get(c0):
                if use_in is True:
                    x = xin[:, c0:c0+LNC].astype(F32)
                else:
                    x = jnp.where(use_in, xin[:, c0:c0+LNC].astype(F32), xs[pa, :, c0:c0+LNC])
                xs[pa, :, c0:c0+LNC] = x
                return x
            ln_to(xna, get)

        def ln_f(pf):
            ln_to(xnf, lambda c0: xs[pf, :, c0:c0+LNC])

        def wo_stage(pf):
            xs[pf] += lax.dot_general(wot[:, 0:D], os_[:, 0:D], NT, preferred_element_type=F32)

        def qkv_stage(pa, la):
            for c in range(5):
                kb[pa, c, 0:HALO, :] = kt[la, c]
                vb[pa, c, 0:HALO, :] = vt[la, c]
            qkv = lax.dot_general(xna[:, 0:D], wqt[:, 0:D], NT, preferred_element_type=F32)
            lane = lax.broadcasted_iota(jnp.int32, (TM, 128), 1)
            qs[pa, :, 0:512] = qkv[:, 0:512] * qscale
            t4 = qkv[:, 512:640]
            qs[pa, :, 512:640] = jnp.where(lane < 64, t4 * qscale, 0.0)
            for c in range(5):
                kk = qkv[:, 640+c*128:640+(c+1)*128] if c < 4 else pltpu.roll(t4, 64, 1)
                vv = qkv[:, 1152+c*128:1152+(c+1)*128]
                kb[pa, c, HALO:, :] = kk
                vb[pa, c, HALO:, :] = vv
                kt[la, c] = kk[TM-HALO:, :]
                vt[la, c] = vv[TM-HALO:, :]

        def first_block_halo(pa):
            for c in range(5):
                kb[pa, c, 0:HALO, :] = jnp.zeros((HALO, 128), F32)
                vb[pa, c, 0:HALO, :] = jnp.broadcast_to(vb[pa, c, HALO:HALO+1, :], (HALO, 128))

        def att_tile(pa, r0, rt, mask_base):
            q = [qs[pa, pl.ds(r0, rt), c*128:(c+1)*128] for c in range(5)]
            lg = []
            for w in range(NW):
                acc = None
                for c in range(5):
                    kk = kb[pa, c, pl.ds(r0 + HALO - DIL*w, rt), :]
                    p = q[c] * kk
                    acc = p if acc is None else acc + p
                acc = acc + pltpu.roll(acc, 64, 1)
                acc = acc + pltpu.roll(acc, 32, 1)
                if mask_base is not None and w > 0:
                    pos = mask_base + lax.broadcasted_iota(jnp.int32, (rt, 128), 0)
                    acc = jnp.where(pos >= DIL*w, acc, -1e9 * LOG2E)
                lg.append(acc)
            mx = lg[0]
            for w in range(1, NW): mx = jnp.maximum(mx, lg[w])
            e = [jnp.exp2(a - mx) for a in lg]
            sm = e[0]
            for w in range(1, NW): sm = sm + e[w]
            inv = 1.0 / sm
            for c in range(5):
                acc = None
                for w in range(NW):
                    vv = vb[pa, c, pl.ds(r0 + HALO - DIL*w, rt), :]
                    t = e[w] * vv
                    acc = t if acc is None else acc + t
                os_[pl.ds(r0, rt), c*128:(c+1)*128] = (acc * inv).astype(BF16)

        def att_rows(pa, base, n, rt, pos0):
            if 'noatt' in ablate: return
            att_tile(pa, base, HALO, pos0)
            r = HALO
            while r < n:
                t = min(rt, n - r)
                att_tile(pa, base + r, t, None)
                r += t

        def ffn_chunk(pf, f):
            xn = xnf[:, 0:D]
            for j in range(FC // FS):
                g = jnp.dot(xn, wg[f, :, j*FS:(j+1)*FS], preferred_element_type=F32)
                u = jnp.dot(xn, wu[f, :, j*FS:(j+1)*FS], preferred_element_type=F32)
                h = (_gelu(g) * u).astype(BF16)
                xs[pf] += lax.dot_general(wd[f, :, j*FS:(j+1)*FS], h, NT, preferred_element_type=F32)

        pa = s % 2
        pf = 1 - pa
        la = (s // 2) % 2
        ab = blk_of(s)

        @pl.when(s == 0)
        def _():
            prep()
            kt[...] = jnp.zeros(kt.shape, F32)
            vt[...] = jnp.zeros(vt.shape, F32)
            ln_a(0, x_ref, True)
            qkv_stage(0, 0)
            first_block_halo(0)
            prep_wo()

        @pl.when(s == 0)
        def _():
            ln_a(1, x1_ref, True)
            if 'attlast' in ablate:
                qkv_stage(1, 0)
                att_rows(0, 0, TM, RTP, 0)
            else:
                att_rows(0, 0, TM, RTP, 0)
                qkv_stage(1, 0)

        @pl.when(jnp.logical_and(s > 1, s < NSLOT - 1))
        def _():
            ln_a(pa, x_ref, la == 0)
            wo_stage(pf)
            qkv_stage(pa, la)
            ln_f(pf)

        @pl.when(jnp.logical_or(s == 1, s == NSLOT - 1))
        def _():
            wo_stage(pf)
            ln_f(pf)

        @pl.when(s == 2)
        def _():
            first_block_halo(0)

        @pl.when(s > 0)
        def _():
            def body(f, _):
                @pl.when(s == 1)
                def _():
                    for ff in range(NF):
                        @pl.when(f == ff)
                        def _():
                            cp_g(ff).wait(); cp_u(ff).wait(); cp_d(ff).wait()
                ffn_chunk(pf, f)
                base = pl.multiple_of(f * PR, PR)
                att_rows(pa, base, PR, RT, ab * TM + base)
                return 0
            lax.fori_loop(0, NF, body, 0)

        @pl.when(jnp.logical_and(s > 0, ((s - 1) // 2) % 2 == 1))
        def _():
            o_ref[...] = xs[pf].astype(o_ref.dtype)

    def x_map(s):
        la = (s // 2) % 2
        b = jnp.where(la == 0, blk_of(s), 2 * (s // 4) + 1)
        return (0, jnp.clip(b, 0, NB - 1))

    def o_map(s):
        fidx = jnp.maximum(s - 1, 0)
        b = 2 * (fidx // 4) + jnp.where(fidx % 4 == 3, 1, 0)
        return (0, b)

    def fn(A_x, A_wqkv, A_wo, B_x, B_w_gate, B_w_up, B_w_down):
        xT = A_x.reshape(S, D).T
        out = pl.pallas_call(
            kernel,
            grid=(NSLOT,),
            in_specs=[pl.BlockSpec((D, TM), x_map), pl.BlockSpec((D, TM), lambda s: (0, 1))] + [pl.BlockSpec(memory_space=pltpu.HBM)] * 5,
            out_specs=pl.BlockSpec((D, TM), o_map),
            out_shape=jax.ShapeDtypeStruct((D, S), BF16),
            scratch_shapes=[
                pltpu.VMEM((D, 3 * D), BF16), pltpu.VMEM((D, D), BF16),
                pltpu.VMEM((5, 1792, 128), F32),
                pltpu.VMEM((1792, 640), BF16), pltpu.VMEM((D, 640), BF16),
                pltpu.VMEM((NF, D, FC), BF16), pltpu.VMEM((NF, D, FC), BF16), pltpu.VMEM((NF, D, FC), BF16),
                pltpu.VMEM((2, D, TM), F32), pltpu.VMEM((TM, 640), BF16), pltpu.VMEM((TM, 640), BF16),
                pltpu.VMEM((2, TM, 640), F32),
                pltpu.VMEM((2, 5, TM + HALO, 128), F32), pltpu.VMEM((2, 5, TM + HALO, 128), F32),
                pltpu.VMEM((2, 5, HALO, 128), F32), pltpu.VMEM((2, 5, HALO, 128), F32),
                pltpu.VMEM((TM, 640), BF16),
                pltpu.SemaphoreType.DMA((2 + 3 * NF,)),
            ],
            compiler_params=pltpu.CompilerParams(dimension_semantics=("arbitrary",), vmem_limit_bytes=100 * 1024 * 1024),
        )(xT, xT, A_wqkv, A_wo, B_w_gate, B_w_up, B_w_down.T)
        return out.T.reshape(1, S, D)
    return fn


_fn = make_kernel(RTP=128)


@jax.jit
def pallas_interleave_layers__sliding_local_dilated__glu_gated_geglu__prompt_kernel(
    A_x: jax.Array,
    A_wqkv: jax.Array,
    A_wo: jax.Array,
    B_x: jax.Array,
    B_w_gate: jax.Array,
    B_w_up: jax.Array,
    B_w_down: jax.Array,
):
    return _fn(A_x, A_wqkv, A_wo, B_x, B_w_gate, B_w_up, B_w_down)
```

```python
import functools
import numpy as np
import jax
import jax.numpy as jnp
from jax import lax
import jax.experimental.pallas as pl
import jax.experimental.pallas.tpu as pltpu

S, D, F, H, DH = 2048, 576, 4608, 32, 18
NW, DIL = 8, 2
HALO = 16
LOG2E = 1.4426950408889634
NT = (((1,), (1,)), ((), ()))
F32, BF16 = jnp.float32, jnp.bfloat16

def _ln_t(x):
    m = jnp.sum(x, axis=0, keepdims=True) * (1.0 / D)
    xc = x - m
    v = jnp.sum(xc * xc, axis=0, keepdims=True) * (1.0 / D)
    return (xc * lax.rsqrt(v + 1e-5)).astype(BF16)

def _gelu(g):
    c = np.float32(np.sqrt(2 / np.pi))
    inner = g * (c + (c * 0.044715) * (g * g))
    hg = 0.5 * g
    return hg + hg * jnp.tanh(inner)

def make_kernel(TM=512, FC=1152, FS=1152, RT=16, RTP=128, LNC=128, KPAD=16, DMAC=4, XPAD=0, QPAD=0, ablate=''):
    NB = S // TM
    NF = F // FC
    NSLOT = 2 * NB + 1
    PR = TM // NF

    def blk_of(a):
        return 2 * (a // 4) + a % 2

    def kernel(x_hbm, wqkv_hbm, wo_hbm, wg_hbm, wu_hbm, wd_hbm, o_ref,
               xin, wraw, woraw, t32, wqt, wot, wg, wu, wd, xs, xna, xnf, qs, kb, vb, kt, vt, os_, sems, sems2):
        s = pl.program_id(0)
        def cp_qkv(c):
            n = 128 if c < 4 else 64
            return pltpu.make_async_copy(wqkv_hbm.at[pl.ds(c*128, n), :], wraw.at[pl.ds(c*128, n), :], sems2.at[c])
        def cp_x(b): return pltpu.make_async_copy(x_hbm.at[:, pl.ds(b*TM, TM)], xin.at[b], sems2.at[5+b])
        def cp_o(): return pltpu.make_async_copy(wo_hbm, woraw, sems.at[1])
        def cp_g(f): return pltpu.make_async_copy(wg_hbm.at[:, pl.ds(f*FC, FC)], wg.at[f], sems.at[2+3*f])
        def cp_u(f): return pltpu.make_async_copy(wu_hbm.at[:, pl.ds(f*FC, FC)], wu.at[f], sems.at[3+3*f])
        def cp_d(f): return pltpu.make_async_copy(wd_hbm.at[:, pl.ds(f*FC, FC)], wd.at[f], sems.at[4+3*f])

        qscale = (DH ** -0.5) * LOG2E

        def prep():
            cp_x(0).start()
            for c in range(5): cp_qkv(c).start()
            cp_x(1).start(); cp_o().start()
            kt[...] = jnp.zeros(kt.shape, F32)
            vt[...] = jnp.zeros(vt.shape, F32)
            wqt[1728:1792, :] = jnp.zeros((64, 640), BF16)
            cp_x(0).wait()
            ln_a(0, xin.at[0], True, xna)
            def dest(p, d):
                if p == 0: return d * 32
                if p == 1: return 576 + (d - 16) * 32 if d >= 16 else 640 + d * 32
                return 1152 + d * 32
            for c in range(5):
                cp_qkv(c).wait()
                kw = 128 if c < 4 else 64
                for j in range(14):
                    nw = 128 if j < 13 else 64
                    blk = wraw[c*128:c*128+kw, j*128:j*128+nw].astype(F32)
                    if kw < 128: blk = jnp.concatenate([blk, jnp.zeros((128-kw, nw), F32)], axis=0)
                    if nw < 128: blk = jnp.concatenate([blk, jnp.zeros((128, 128-nw), F32)], axis=1)
                    t32[c, j*128:(j+1)*128, :] = blk.T
                for p in range(3):
                    for d in range(DH):
                        rows = t32[c, pl.ds(p * D + d, H, stride=DH), :]
                        r0 = dest(p, d)
                        wqt[r0:r0+H, c*128:(c+1)*128] = rows.astype(BF16)
                if c == DMAC:
                    for f in range(NF):
                        cp_g(f).start(); cp_u(f).start(); cp_d(f).start()
                    for b in range(2, NB): cp_x(b).start()

        def prep_wo():
            cp_o().wait()
            for c in range(5):
                nw = 128 if c < 4 else 64
                blk = woraw[:, c*128:c*128+nw].astype(F32)
                if nw < 128: blk = jnp.concatenate([blk, jnp.zeros((D, 128-nw), F32)], axis=1)
                t32[c, 0:D, :] = blk
            for c in range(5):
                parts = [t32[c, pl.ds(d, H, stride=DH), :] for d in range(DH)] + [jnp.zeros((64, 128), F32)]
                wp = jnp.concatenate(parts, axis=0)
                res = wp.T.astype(BF16)
                nw = 128 if c < 4 else 64
                wot[c*128:c*128+nw, :] = res[:nw]

        dz = jnp.minimum(s, 0)

        def ln_to(dst, first, p):
            for c0 in range(0, TM, LNC):
                x = first(c0)
                m = jnp.sum(x, axis=0, keepdims=True) * (1.0 / D)
                if 'reload' in ablate:
                    x = xs[p, :, pl.ds(pl.multiple_of(c0 + dz * 128, 128), LNC)]
                xc = x - m
                v = jnp.sum(xc * xc, axis=0, keepdims=True) * (1.0 / D)
                r = lax.rsqrt(v + 1e-5)
                if 'reload' in ablate:
                    x = xs[p, :, pl.ds(pl.multiple_of(c0 + dz * 256, 128), LNC)]
                    xc = x - m
                dst[c0:c0+LNC, 0:D] = (xc * r).astype(BF16).T

        def ln_a(pa, xin, use_in, dst):
            def first(c0):
                if use_in is True:
                    x = xin[:, c0:c0+LNC].astype(F32)
                else:
                    x = jnp.where(use_in, xin[:, c0:c0+LNC].astype(F32), xs[pa, :, c0:c0+LNC])
                xs[pa, :, c0:c0+LNC] = x
                return x
            ln_to(dst, first, pa)

        def ln_f(pf):
            ln_to(xnf, lambda c0: xs[pf, :, c0:c0+LNC], pf)

        def wo_stage(pf):
            xs[pf] += lax.dot_general(wot[:, 0:D], os_[:, 0:D], NT, preferred_element_type=F32)

        def qkv_stage(pa, la, src):
            for c in range(5):
                kb[pa, c, 0:HALO, :] = kt[la, c]
                vb[pa, c, 0:HALO, :] = vt[la, c]
            qkv = lax.dot_general(src[:, 0:D], wqt[:, 0:D], NT, preferred_element_type=F32)
            lane = lax.broadcasted_iota(jnp.int32, (TM, 128), 1)
            qs[pa, :, 0:512] = qkv[:, 0:512] * qscale
            t4 = qkv[:, 512:640]
            qs[pa, :, 512:640] = jnp.where(lane < 64, t4 * qscale, 0.0)
            for c in range(5):
                kk = qkv[:, 640+c*128:640+(c+1)*128] if c < 4 else pltpu.roll(t4, 64, 1)
                vv = qkv[:, 1152+c*128:1152+(c+1)*128]
                kb[pa, c, HALO:HALO+TM, :] = kk
                vb[pa, c, HALO:HALO+TM, :] = vv
                kt[la, c] = kk[TM-HALO:, :]
                vt[la, c] = vv[TM-HALO:, :]

        def first_block_halo(pa):
            for c in range(5):
                kb[pa, c, 0:HALO, :] = jnp.zeros((HALO, 128), F32)
                vb[pa, c, 0:HALO, :] = jnp.broadcast_to(vb[pa, c, HALO:HALO+1, :], (HALO, 128))

        def att_tile(pa, r0, rt, mask_base):
            q = [qs[pa, pl.ds(r0, rt), c*128:(c+1)*128] for c in range(5)]
            lg = []
            for w in range(NW):
                acc = None
                for c in range(5):
                    kk = kb[pa, c, pl.ds(r0 + HALO - DIL*w, rt), :]
                    p = q[c] * kk
                    acc = p if acc is None else acc + p
                acc = acc + pltpu.roll(acc, 64, 1)
                acc = acc + pltpu.roll(acc, 32, 1)
                if mask_base is not None and w > 0:
                    pos = mask_base + lax.broadcasted_iota(jnp.int32, (rt, 128), 0)
                    acc = jnp.where(pos >= DIL*w, acc, -1e9 * LOG2E)
                lg.append(acc)
            mx = lg[0]
            for w in range(1, NW): mx = jnp.maximum(mx, lg[w])
            e = [jnp.exp2(a - mx) for a in lg]
            sm = e[0]
            for w in range(1, NW): sm = sm + e[w]
            inv = 1.0 / sm
            for c in range(5):
                acc = None
                for w in range(NW):
                    vv = vb[pa, c, pl.ds(r0 + HALO - DIL*w, rt), :]
                    t = e[w] * vv
                    acc = t if acc is None else acc + t
                os_[pl.ds(r0, rt), c*128:(c+1)*128] = (acc * inv).astype(BF16)

        def att_rows(pa, base, n, rt, pos0):
            if 'noatt' in ablate: return
            att_tile(pa, base, HALO, pos0)
            r = HALO
            while r < n:
                t = min(rt, n - r)
                att_tile(pa, base + r, t, None)
                r += t

        def ffn_chunk(pf, f):
            xn = xnf[:, 0:D]
            for j in range(FC // FS):
                g = jnp.dot(xn, wg[f, :, j*FS:(j+1)*FS], preferred_element_type=F32)
                u = jnp.dot(xn, wu[f, :, j*FS:(j+1)*FS], preferred_element_type=F32)
                h = (_gelu(g) * u).astype(BF16)
                xs[pf] += lax.dot_general(wd[f, :, j*FS:(j+1)*FS], h, NT, preferred_element_type=F32)

        pa = s % 2
        pf = 1 - pa
        la = (s // 2) % 2
        ab = blk_of(s)

        @pl.when(s == 0)
        @jax.named_scope("P0")
        def _():
            prep()
            cp_x(1).wait()
            qkv_stage(0, 0, xna)
            ln_a(1, xin.at[1], True, xnf)
            first_block_halo(0)
            prep_wo()

        @pl.when(s == 0)
        @jax.named_scope("P1")
        def _():
            if 'attlast' in ablate:
                qkv_stage(1, 0, xnf)
                att_rows(0, 0, TM, RTP, 0)
            else:
                att_rows(0, 0, TM, RTP, 0)
                qkv_stage(1, 0, xnf)

        for b in range(2, NB):
            @pl.when(s == 2 * b)
            def _():
                cp_x(b).wait()

        @pl.when(jnp.logical_and(s > 1, s < NSLOT - 1))
        @jax.named_scope("R")
        def _():
            ln_a(pa, xin.at[jnp.minimum(ab, NB - 1)], la == 0, xna)
            wo_stage(pf)
            qkv_stage(pa, la, xna)
            ln_f(pf)

        @pl.when(jnp.logical_or(s == 1, s == NSLOT - 1))
        @jax.named_scope("RS")
        def _():
            wo_stage(pf)
            ln_f(pf)

        @pl.when(s == 2)
        def _():
            first_block_halo(0)

        @pl.when(s > 0)
        @jax.named_scope("LOOP")
        def _():
            def body(f, _):
                @pl.when(s == 1)
                def _():
                    for ff in range(NF):
                        @pl.when(f == ff)
                        def _():
                            cp_g(ff).wait(); cp_u(ff).wait(); cp_d(ff).wait()
                ffn_chunk(pf, f)
                base = pl.multiple_of(f * PR, PR)
                att_rows(pa, base, PR, RT, ab * TM + base)
                return 0
            lax.fori_loop(0, NF, body, 0)

        @pl.when(jnp.logical_and(s > 0, ((s - 1) // 2) % 2 == 1))
        def _():
            o_ref[...] = xs[pf].astype(o_ref.dtype)

    def x_map(s):
        la = (s // 2) % 2
        b = jnp.where(la == 0, blk_of(s), 2 * (s // 4) + 1)
        return (0, jnp.clip(b, 0, NB - 1))

    def o_map(s):
        fidx = jnp.maximum(s - 1, 0)
        b = 2 * (fidx // 4) + jnp.where(fidx % 4 == 3, 1, 0)
        return (0, b)

    def fn(A_x, A_wqkv, A_wo, B_x, B_w_gate, B_w_up, B_w_down):
        xT = A_x.reshape(S, D).T
        out = pl.pallas_call(
            kernel,
            grid=(NSLOT,),
            in_specs=[pl.BlockSpec(memory_space=pltpu.HBM)] * 6,
            out_specs=pl.BlockSpec((D, TM), o_map),
            out_shape=jax.ShapeDtypeStruct((D, S), BF16),
            scratch_shapes=[
                pltpu.VMEM((NB, D, TM), BF16), pltpu.VMEM((D, 3 * D), BF16), pltpu.VMEM((D, D), BF16),
                pltpu.VMEM((5, 1792, 128), F32),
                pltpu.VMEM((1792, 640), BF16), pltpu.VMEM((D, 640), BF16),
                pltpu.VMEM((NF, D, FC), BF16), pltpu.VMEM((NF, D, FC), BF16), pltpu.VMEM((NF, D, FC), BF16),
                pltpu.VMEM((2, D, TM), F32), pltpu.VMEM((TM, 640), BF16), pltpu.VMEM((TM, 640), BF16),
                pltpu.VMEM((2, TM, 640), F32),
                pltpu.VMEM((2, 5, TM + HALO + KPAD, 128), F32), pltpu.VMEM((2, 5, TM + HALO + KPAD, 128), F32),
                pltpu.VMEM((2, 5, HALO, 128), F32), pltpu.VMEM((2, 5, HALO, 128), F32),
                pltpu.VMEM((TM, 640), BF16),
                pltpu.SemaphoreType.DMA((2 + 3 * NF,)), pltpu.SemaphoreType.DMA((5 + NB,)),
            ],
            compiler_params=pltpu.CompilerParams(dimension_semantics=("arbitrary",), vmem_limit_bytes=100 * 1024 * 1024),
        )(xT, A_wqkv, A_wo, B_w_gate, B_w_up, B_w_down.T)
        return out.T.reshape(1, S, D)
    return fn


_fn = make_kernel(RTP=128, ablate='attlast')


@jax.jit
def pallas_interleave_layers__sliding_local_dilated__glu_gated_geglu__prompt_kernel(
    A_x: jax.Array,
    A_wqkv: jax.Array,
    A_wo: jax.Array,
    B_x: jax.Array,
    B_w_gate: jax.Array,
    B_w_up: jax.Array,
    B_w_down: jax.Array,
):
    return _fn(A_x, A_wqkv, A_wo, B_x, B_w_gate, B_w_up, B_w_down)
```

```python
import functools
import numpy as np
import jax
import jax.numpy as jnp
from jax import lax
import jax.experimental.pallas as pl
import jax.experimental.pallas.tpu as pltpu

S, D, F, H, DH = 2048, 576, 4608, 32, 18
NW, DIL = 8, 2
HALO = 16
LOG2E = 1.4426950408889634
NT = (((1,), (1,)), ((), ()))
F32, BF16 = jnp.float32, jnp.bfloat16

def _ln_t(x):
    m = jnp.sum(x, axis=0, keepdims=True) * (1.0 / D)
    xc = x - m
    v = jnp.sum(xc * xc, axis=0, keepdims=True) * (1.0 / D)
    return (xc * lax.rsqrt(v + 1e-5)).astype(BF16)

def _gelu(g):
    c = np.float32(np.sqrt(2 / np.pi))
    inner = g * (c + (c * 0.044715) * (g * g))
    hg = 0.5 * g
    return hg + hg * jnp.tanh(inner)

def make_kernel(TM=512, FC=1536, GS=512, PRB=32, TIE=0, U32=1, RT=16, RTP=128, LNC=128, KPAD=16, DMAC=4, XPAD=0, QPAD=0, ablate=''):
    NB = S // TM
    NF = F // FC
    NSLOT = 2 * NB + 1
    PR = -(-TM // NF // RT) * RT
    HT = TM // 2
    fs = GS // 2
    NG = FC // GS

    def blk_of(a):
        return 2 * (a // 4) + a % 2

    def kernel(x_hbm, wqkv_hbm, wo_hbm, wg_hbm, wu_hbm, wd_hbm, o_ref,
               xin, wraw, woraw, t32, wqt, wot, wg, wu, wd, tg, td, xs, xna, xn1, xnf, sa, qs, kb, vb, kt, vt, os_, sems, sems2, flag):
        s = pl.program_id(0)
        def cp_qkv(c):
            n = 128 if c < 4 else 64
            return pltpu.make_async_copy(wqkv_hbm.at[pl.ds(c*128, n), :], wraw.at[pl.ds(c*128, n), :], sems2.at[c])
        def cp_x(b): return pltpu.make_async_copy(x_hbm.at[:, pl.ds(b*TM, TM)], xin.at[b], sems2.at[5+b])
        def cp_o(): return pltpu.make_async_copy(wo_hbm, woraw, sems.at[1])
        def cp_g(f): return pltpu.make_async_copy(wg_hbm.at[:, pl.ds(f*FC, FC)], wg.at[f], sems.at[2+3*f])
        def cp_u(f): return pltpu.make_async_copy(wu_hbm.at[:, pl.ds(f*FC, FC)], wu.at[f], sems.at[3+3*f])
        def cp_d(f): return pltpu.make_async_copy(wd_hbm.at[:, pl.ds(f*FC, FC)], wd.at[f], sems.at[4+3*f])

        qscale = (DH ** -0.5) * LOG2E

        def prep():
            cp_x(0).start()
            for c in range(5): cp_qkv(c).start()
            cp_x(1).start(); cp_o().start()
            kt[...] = jnp.zeros(kt.shape, F32)
            vt[...] = jnp.zeros(vt.shape, F32)
            wqt[1728:1792, :] = jnp.zeros((64, 640), BF16)
            cp_x(0).wait()
            ln_a(0, xin.at[0], True, xna)
            def dest(p, d):
                if p == 0: return d * 32
                if p == 1: return 576 + (d - 16) * 32 if d >= 16 else 640 + d * 32
                return 1152 + d * 32
            for c in range(5):
                cp_qkv(c).wait()
                kw = 128 if c < 4 else 64
                for j in range(14):
                    nw = 128 if j < 13 else 64
                    blk = wraw[c*128:c*128+kw, j*128:j*128+nw].astype(F32)
                    if kw < 128: blk = jnp.concatenate([blk, jnp.zeros((128-kw, nw), F32)], axis=0)
                    if nw < 128: blk = jnp.concatenate([blk, jnp.zeros((128, 128-nw), F32)], axis=1)
                    t32[c, j*128:(j+1)*128, :] = blk.T
                for p in range(3):
                    for d in range(DH):
                        rows = t32[c, pl.ds(p * D + d, H, stride=DH), :]
                        r0 = dest(p, d)
                        wqt[r0:r0+H, c*128:(c+1)*128] = rows.astype(BF16)
                if c == DMAC:
                    for f in range(NF):
                        cp_g(f).start(); cp_u(f).start(); cp_d(f).start()
                    for b in range(2, NB): cp_x(b).start()

        def prep_wo():
            cp_o().wait()
            for c in range(5):
                nw = 128 if c < 4 else 64
                blk = woraw[:, c*128:c*128+nw].astype(F32)
                if nw < 128: blk = jnp.concatenate([blk, jnp.zeros((D, 128-nw), F32)], axis=1)
                t32[c, 0:D, :] = blk
            for c in range(5):
                parts = [t32[c, pl.ds(d, H, stride=DH), :] for d in range(DH)] + [jnp.zeros((64, 128), F32)]
                wp = jnp.concatenate(parts, axis=0)
                res = wp.T.astype(BF16)
                nw = 128 if c < 4 else 64
                wot[c*128:c*128+nw, :] = res[:nw]

        dz = jnp.minimum(s, 0)

        def ln_to(dst, first, p):
            for c0 in range(0, TM, LNC):
                x = first(c0)
                m = jnp.sum(x, axis=0, keepdims=True) * (1.0 / D)
                if 'reload' in ablate:
                    x = xs[p, :, pl.ds(pl.multiple_of(c0 + dz * 128, 128), LNC)]
                xc = x - m
                v = jnp.sum(xc * xc, axis=0, keepdims=True) * (1.0 / D)
                r = lax.rsqrt(v + 1e-5)
                if 'reload' in ablate:
                    x = xs[p, :, pl.ds(pl.multiple_of(c0 + dz * 256, 128), LNC)]
                    xc = x - m
                dst[c0:c0+LNC, 0:D] = (xc * r).astype(BF16).T

        def ln_a(pa, xin, use_in, dst):
            def first(c0):
                if use_in is True:
                    x = xin[:, c0:c0+LNC].astype(F32)
                else:
                    x = jnp.where(use_in, xin[:, c0:c0+LNC].astype(F32), xs[pa, :, c0:c0+LNC])
                xs[pa, :, c0:c0+LNC] = x
                return x
            ln_to(dst, first, pa)

        def ln_f(pf):
            def norm(c0):
                x = xs[pf, :, c0:c0+LNC]
                m = jnp.sum(x, axis=0, keepdims=True) * (1.0 / D)
                xc = x - m
                v = jnp.sum(xc * xc, axis=0, keepdims=True) * (1.0 / D)
                return xc * lax.rsqrt(v + 1e-5)
            for c0 in range(0, HT, LNC):
                n1 = norm(c0); n2 = norm(HT + c0)
                a11 = n1[0:256]; a12 = n1[256:512]; a21 = n2[0:256]; a22 = n2[256:512]
                for j, val in enumerate([a11 + a22, a21 + a22, a11, a22, a11 + a12, a21 - a11, a12 - a22]):
                    sa[j, rs(c0, LNC), :] = pk(val.astype(BF16).T)
                xnf[c0:c0+LNC, 0:64] = n1[512:576].astype(BF16).T
                xnf[HT+c0:HT+c0+LNC, 0:64] = n2[512:576].astype(BF16).T

        def wo_stage(pf):
            xs[pf] += lax.dot_general(wot[:, 0:D], os_[:, 0:D], NT, preferred_element_type=F32)

        def qkv_stage(pa, la, src):
            for c in range(5):
                kb[pa, c, 0:HALO, :] = kt[la, c]
                vb[pa, c, 0:HALO, :] = vt[la, c]
            qkv = lax.dot_general(src[:, 0:D], wqt[:, 0:D], NT, preferred_element_type=F32)
            lane = lax.broadcasted_iota(jnp.int32, (TM, 128), 1)
            qs[pa, :, 0:512] = qkv[:, 0:512] * qscale
            t4 = qkv[:, 512:640]
            qs[pa, :, 512:640] = jnp.where(lane < 64, t4 * qscale, 0.0)
            for c in range(5):
                kk = qkv[:, 640+c*128:640+(c+1)*128] if c < 4 else pltpu.roll(t4, 64, 1)
                vv = qkv[:, 1152+c*128:1152+(c+1)*128]
                kb[pa, c, HALO:HALO+TM, :] = kk
                vb[pa, c, HALO:HALO+TM, :] = vv
                kt[la, c] = kk[TM-HALO:, :]
                vt[la, c] = vv[TM-HALO:, :]

        def first_block_halo(pa):
            for c in range(5):
                kb[pa, c, 0:HALO, :] = jnp.zeros((HALO, 128), F32)
                vb[pa, c, 0:HALO, :] = jnp.broadcast_to(vb[pa, c, HALO:HALO+1, :], (HALO, 128))

        def att_tile(pa, r0, rt, mask_base):
            q = [qs[pa, pl.ds(r0, rt), c*128:(c+1)*128] for c in range(5)]
            lg = []
            for w in range(NW):
                acc = None
                for c in range(5):
                    kk = kb[pa, c, pl.ds(r0 + HALO - DIL*w, rt), :]
                    p = q[c] * kk
                    acc = p if acc is None else acc + p
                acc = acc + pltpu.roll(acc, 64, 1)
                acc = acc + pltpu.roll(acc, 32, 1)
                if mask_base is not None and w > 0:
                    pos = mask_base + lax.broadcasted_iota(jnp.int32, (rt, 128), 0)
                    acc = jnp.where(pos >= DIL*w, acc, -1e9 * LOG2E)
                lg.append(acc)
            mx = lg[0]
            for w in range(1, NW): mx = jnp.maximum(mx, lg[w])
            e = [jnp.exp2(a - mx) for a in lg]
            sm = e[0]
            for w in range(1, NW): sm = sm + e[w]
            inv = 1.0 / sm
            res = []
            for c in range(5):
                acc = None
                for w in range(NW):
                    vv = vb[pa, c, pl.ds(r0 + HALO - DIL*w, rt), :]
                    t = e[w] * vv
                    acc = t if acc is None else acc + t
                o = (acc * inv).astype(BF16)
                os_[pl.ds(r0, rt), c*128:(c+1)*128] = o
                res.append(o)
            return res

        def att_rows(pa, base, n, rt, pos0):
            if 'noatt' in ablate: return
            att_tile(pa, base, HALO, pos0)
            r = HALO
            while r < n:
                t = min(rt, n - r)
                att_tile(pa, base + r, t, None)
                r += t

        def pk(x):
            return pltpu.bitcast(x, jnp.uint32) if U32 else x
        def upk(x):
            return pltpu.bitcast(x, BF16) if U32 else x
        def rs(r0, n):
            return slice(r0 // 2, (r0 + n) // 2) if U32 else slice(r0, r0 + n)
        def ra(n):
            return slice(0, n // 2) if U32 else slice(0, n)

        def dot(a, b): return jnp.dot(a, b, preferred_element_type=F32)
        def dnt(a, b): return lax.dot_general(a, b, NT, preferred_element_type=F32)

        def ffn_prep_gu(f, cs):
            for r in range(0, 256, PRB):
                r1 = slice(r, r + PRB); r2 = slice(256 + r, 256 + r + PRB)
                b11 = wg[f, r1, cs].astype(F32); b12 = wu[f, r1, cs].astype(F32)
                b21 = wg[f, r2, cs].astype(F32); b22 = wu[f, r2, cs].astype(F32)
                tg[f, 0, rs(r, PRB), cs] = pk((b11 + b22).astype(BF16))
                tg[f, 1, rs(r, PRB), cs] = pk((b12 - b22).astype(BF16))
                tg[f, 2, rs(r, PRB), cs] = pk((b21 - b11).astype(BF16))
                tg[f, 3, rs(r, PRB), cs] = pk((b11 + b12).astype(BF16))
                tg[f, 4, rs(r, PRB), cs] = pk((b21 + b22).astype(BF16))

        def ffn_prep_d(f, k1, k2, ko):
            for r in range(0, 288, PRB):
                n = min(PRB, 288 - r)
                r1 = slice(r, r + n); r2 = slice(288 + r, 288 + r + n)
                a11 = wd[f, r1, k1].astype(F32); a12 = wd[f, r1, k2].astype(F32)
                a21 = wd[f, r2, k1].astype(F32); a22 = wd[f, r2, k2].astype(F32)
                td[f, 0, rs(r, n), ko] = pk((a11 + a22).astype(BF16))
                td[f, 1, rs(r, n), ko] = pk((a21 + a22).astype(BF16))
                td[f, 2, rs(r, n), ko] = pk((a11 + a12).astype(BF16))
                td[f, 3, rs(r, n), ko] = pk((a21 - a11).astype(BF16))
                td[f, 4, rs(r, n), ko] = pk((a12 - a22).astype(BF16))

        def ffn_prep(f):
            def pbody(c, _):
                ffn_prep_gu(f, pl.ds(pl.multiple_of(c * 128, 128), 128))
                return 0
            lax.fori_loop(0, FC // 128, pbody, 0)
            def dbody(c, _):
                gi = c // (fs // 128); cc = c % (fs // 128)
                k1 = pl.ds(pl.multiple_of(gi * GS + cc * 128, 128), 128)
                k2 = pl.ds(pl.multiple_of(gi * GS + fs + cc * 128, 128), 128)
                ko = pl.ds(pl.multiple_of(c * 128, 128), 128)
                ffn_prep_d(f, k1, k2, ko)
                return 0
            lax.fori_loop(0, FC // 256, dbody, 0)

        def ffn_up(f, gi):
            hs = {}
            for kh in range(2):
                cs = slice(gi * GS + kh * fs, gi * GS + (kh + 1) * fs)
                m1 = dot(upk(sa[0]), upk(tg[f, 0, :, cs]))
                m2 = dot(upk(sa[1]), wg[f, 0:256, cs])
                m3 = dot(upk(sa[2]), upk(tg[f, 1, :, cs]))
                m4 = dot(upk(sa[3]), upk(tg[f, 2, :, cs]))
                m5 = dot(upk(sa[4]), wu[f, 256:512, cs])
                m6 = dot(upk(sa[5]), upk(tg[f, 3, :, cs]))
                m7 = dot(upk(sa[6]), upk(tg[f, 4, :, cs]))
                tl = xnf[:, 0:64]
                gt = dot(tl, wg[f, 512:576, cs]); ut = dot(tl, wu[f, 512:576, cs])
                g1 = m1 + m4 - m5 + m7 + gt[0:HT]
                u1 = m3 + m5 + ut[0:HT]
                g2 = m2 + m4 + gt[HT:TM]
                u2 = m1 - m2 + m3 + m6 + ut[HT:TM]
                hs[(0, kh)] = _gelu(g1) * u1
                hs[(1, kh)] = _gelu(g2) * u2
            b11, b12, b21, b22 = hs[(0, 0)], hs[(1, 0)], hs[(0, 1)], hs[(1, 1)]
            return [v.astype(BF16) for v in (b11 + b22, b11, b12 - b22, b21 - b11, b22, b11 + b12, b21 + b22)]

        def ffn_down(pf, f, gi, hb):
            ko = slice(gi * fs, (gi + 1) * fs)
            k1 = slice(gi * GS, gi * GS + fs); k2 = slice(gi * GS + fs, (gi + 1) * GS)
            n1 = dnt(upk(td[f, 0, :, ko]), hb[0])
            n2 = dnt(upk(td[f, 1, :, ko]), hb[1])
            n3 = dnt(wd[f, 0:288, k1], hb[2])
            n4 = dnt(wd[f, 288:576, k2], hb[3])
            n5 = dnt(upk(td[f, 2, :, ko]), hb[4])
            n6 = dnt(upk(td[f, 3, :, ko]), hb[5])
            n7 = dnt(upk(td[f, 4, :, ko]), hb[6])
            xs[pf, 0:288, 0:HT] += n1 + n4 - n5 + n7
            xs[pf, 0:288, HT:TM] += n3 + n5
            xs[pf, 288:576, 0:HT] += n2 + n4
            xs[pf, 288:576, HT:TM] += n1 - n2 + n3 + n6

        def ffn_chunk(pf, f, att_parts):
            prev = None
            for gi in range(NG):
                cur = ffn_up(f, gi)
                outs = att_parts[gi]()
                if TIE and outs:
                    z = cur[1][0:RT, 0:128]
                    for o in outs: z = jnp.where(never, o, z)
                    top = jnp.concatenate([z, cur[1][0:RT, 128:]], axis=1) if fs > 128 else z
                    cur[1] = jnp.concatenate([top, cur[1][RT:]], axis=0)
                if prev is not None: ffn_down(pf, f, gi - 1, prev)
                prev = cur
            ffn_down(pf, f, NG - 1, prev)

        @pl.when(s == 0)
        def _():
            flag[0] = 0
        never = flag[0] != 0
        pa = s % 2
        pf = 1 - pa
        la = (s // 2) % 2
        ab = blk_of(s)

        @pl.when(s == 0)
        @jax.named_scope("P0")
        def _():
            prep()
            cp_x(1).wait()
            qkv_stage(0, 0, xna)
            ln_a(1, xin.at[1], True, xn1)
            first_block_halo(0)
            prep_wo()

        @pl.when(s == 0)
        @jax.named_scope("P1")
        def _():
            if 'attlast' in ablate:
                qkv_stage(1, 0, xn1)
                att_rows(0, 0, TM, RTP, 0)
            else:
                att_rows(0, 0, TM, RTP, 0)
                qkv_stage(1, 0, xn1)

        for b in range(2, NB):
            @pl.when(s == 2 * b)
            def _():
                cp_x(b).wait()

        @pl.when(jnp.logical_and(s > 1, s < NSLOT - 1))
        @jax.named_scope("R")
        def _():
            ln_a(pa, xin.at[jnp.minimum(ab, NB - 1)], la == 0, xna)
            wo_stage(pf)
            qkv_stage(pa, la, xna)
            ln_f(pf)

        @pl.when(jnp.logical_or(s == 1, s == NSLOT - 1))
        @jax.named_scope("RS")
        def _():
            wo_stage(pf)
            ln_f(pf)

        @pl.when(s == 2)
        def _():
            first_block_halo(0)

        @pl.when(s > 0)
        @jax.named_scope("LOOP")
        def _():
            def body(f, _):
                @pl.when(s == 1)
                def _():
                    for ff in range(NF):
                        @pl.when(f == ff)
                        def _():
                            cp_g(ff).wait(); cp_u(ff).wait(); cp_d(ff).wait()
                    ffn_prep(f)
                base = pl.multiple_of(jnp.minimum(f * PR, TM - PR), RT)
                tiles = [functools.partial(att_tile, pa, base + r, RT, (ab * TM + base) if r == 0 else None)
                         for r in range(0, PR, RT)]
                nper = -(-len(tiles) // NG)
                def part(j):
                    def run():
                        if 'noatt' in ablate: return []
                        return [o for t in tiles[j*nper:(j+1)*nper] for o in t()]
                    return run
                ffn_chunk(pf, f, [part(j) for j in range(NG)])
                return 0
            lax.fori_loop(0, NF, body, 0)

        @pl.when(jnp.logical_and(s > 0, ((s - 1) // 2) % 2 == 1))
        def _():
            o_ref[...] = xs[pf].astype(o_ref.dtype)

    def x_map(s):
        la = (s // 2) % 2
        b = jnp.where(la == 0, blk_of(s), 2 * (s // 4) + 1)
        return (0, jnp.clip(b, 0, NB - 1))

    def o_map(s):
        fidx = jnp.maximum(s - 1, 0)
        b = 2 * (fidx // 4) + jnp.where(fidx % 4 == 3, 1, 0)
        return (0, b)

    def fn(A_x, A_wqkv, A_wo, B_x, B_w_gate, B_w_up, B_w_down):
        xT = A_x.reshape(S, D).T
        out = pl.pallas_call(
            kernel,
            grid=(NSLOT,),
            in_specs=[pl.BlockSpec(memory_space=pltpu.HBM)] * 6,
            out_specs=pl.BlockSpec((D, TM), o_map),
            out_shape=jax.ShapeDtypeStruct((D, S), BF16),
            scratch_shapes=[
                pltpu.VMEM((NB, D, TM), BF16), pltpu.VMEM((D, 3 * D), BF16), pltpu.VMEM((D, D), BF16),
                pltpu.VMEM((5, 1792, 128), F32),
                pltpu.VMEM((1792, 640), BF16), pltpu.VMEM((D, 640), BF16),
                pltpu.VMEM((NF, D, FC), BF16), pltpu.VMEM((NF, D, FC), BF16), pltpu.VMEM((NF, D, FC), BF16),
                pltpu.VMEM((NF, 5, 128, FC), jnp.uint32) if U32 else pltpu.VMEM((NF, 5, 256, FC), BF16),
                pltpu.VMEM((NF, 5, 144, FC // 2), jnp.uint32) if U32 else pltpu.VMEM((NF, 5, 288, FC // 2), BF16),
                pltpu.VMEM((2, D, TM), F32), pltpu.VMEM((TM, 640), BF16), pltpu.VMEM((TM, 640), BF16), pltpu.VMEM((TM, 128), BF16), pltpu.VMEM((7, HT // 2, 256), jnp.uint32) if U32 else pltpu.VMEM((7, HT, 256), BF16),
                pltpu.VMEM((2, TM, 640), F32),
                pltpu.VMEM((2, 5, TM + HALO + KPAD, 128), F32), pltpu.VMEM((2, 5, TM + HALO + KPAD, 128), F32),
                pltpu.VMEM((2, 5, HALO, 128), F32), pltpu.VMEM((2, 5, HALO, 128), F32),
                pltpu.VMEM((TM, 640), BF16),
                pltpu.SemaphoreType.DMA((2 + 3 * NF,)), pltpu.SemaphoreType.DMA((5 + NB,)), pltpu.SMEM((1,), jnp.int32),
            ],
            compiler_params=pltpu.CompilerParams(dimension_semantics=("arbitrary",), vmem_limit_bytes=112 * 1024 * 1024),
        )(xT, A_wqkv, A_wo, B_w_gate, B_w_up, B_w_down.T)
        return out.T.reshape(1, S, D)
    return fn


_fn = make_kernel(GS=768, ablate='attlast')


@jax.jit
def pallas_interleave_layers__sliding_local_dilated__glu_gated_geglu__prompt_kernel(
    A_x: jax.Array,
    A_wqkv: jax.Array,
    A_wo: jax.Array,
    B_x: jax.Array,
    B_w_gate: jax.Array,
    B_w_up: jax.Array,
    B_w_down: jax.Array,
):
    return _fn(A_x, A_wqkv, A_wo, B_x, B_w_gate, B_w_up, B_w_down)
```

```python
import functools
import numpy as np
import jax
import jax.numpy as jnp
from jax import lax
import jax.experimental.pallas as pl
import jax.experimental.pallas.tpu as pltpu

S, D, F, H, DH = 2048, 576, 4608, 32, 18
NW, DIL = 8, 2
HALO = 16
LOG2E = 1.4426950408889634
NT = (((1,), (1,)), ((), ()))
F32, BF16 = jnp.float32, jnp.bfloat16

def _ln_t(x):
    m = jnp.sum(x, axis=0, keepdims=True) * (1.0 / D)
    xc = x - m
    v = jnp.sum(xc * xc, axis=0, keepdims=True) * (1.0 / D)
    return (xc * lax.rsqrt(v + 1e-5)).astype(BF16)

def _gelu(g):
    c = np.float32(np.sqrt(2 / np.pi))
    inner = g * (c + (c * 0.044715) * (g * g))
    hg = 0.5 * g
    return hg + hg * jnp.tanh(inner)

def make_kernel(TM=512, FC=1536, GS=512, PRB=32, PP=0, UO=1, QS=1, TIE=0, U32=1, RT=16, RTP=128, LNC=128, KPAD=16, DMAC=4, XPAD=0, QPAD=0, ablate=''):
    NB = S // TM
    NF = F // FC
    NSLOT = 2 * NB + 1
    PR = -(-TM // NF // RT) * RT
    HT = TM // 2
    fs = GS // 2
    NG = FC // GS

    def blk_of(a):
        return 2 * (a // 4) + a % 2

    def kernel(x_hbm, wqkv_hbm, wo_hbm, wg_hbm, wu_hbm, wd_hbm, o_ref,
               xin, wraw, woraw, t32, wqt, wot, wg, wu, wd, tg, tu, td, xs, xna, xn1, xnf, sa, sq, xqt, tq, qs, kb, vb, kt, vt, os_, sems, sems2, flag):
        s = pl.program_id(0)
        def cp_qkv(c):
            n = 128 if c < 4 else 64
            return pltpu.make_async_copy(wqkv_hbm.at[pl.ds(c*128, n), :], wraw.at[pl.ds(c*128, n), :], sems2.at[c])
        def cp_x(b): return pltpu.make_async_copy(x_hbm.at[:, pl.ds(b*TM, TM)], xin.at[b], sems2.at[5+b])
        def cp_o(): return pltpu.make_async_copy(wo_hbm, woraw, sems.at[1])
        def cp_g(f): return pltpu.make_async_copy(wg_hbm.at[:, pl.ds(f*FC, FC)], wg.at[f], sems.at[2+3*f])
        def cp_u(f): return pltpu.make_async_copy(wu_hbm.at[:, pl.ds(f*FC, FC)], wu.at[f], sems.at[3+3*f])
        def cp_d(f): return pltpu.make_async_copy(wd_hbm.at[:, pl.ds(f*FC, FC)], wd.at[f], sems.at[4+3*f])

        qscale = (DH ** -0.5) * LOG2E

        def prep():
            cp_x(0).start()
            for c in range(5): cp_qkv(c).start()
            cp_x(1).start(); cp_o().start()
            kt[...] = jnp.zeros(kt.shape, F32)
            vt[...] = jnp.zeros(vt.shape, F32)
            wqt[1728:1792, :] = jnp.zeros((64, 640), BF16)
            cp_x(0).wait()
            (ln_a2(0, xin.at[0], True, sq, xqt) if QS else ln_a(0, xin.at[0], True, xna))
            def dest(p, d):
                if p == 0: return d * 32
                if p == 1: return 576 + (d - 16) * 32 if d >= 16 else 640 + d * 32
                return 1152 + d * 32
            for c in range(5):
                cp_qkv(c).wait()
                kw = 128 if c < 4 else 64
                for j in range(14):
                    nw = 128 if j < 13 else 64
                    blk = wraw[c*128:c*128+kw, j*128:j*128+nw].astype(F32)
                    if kw < 128: blk = jnp.concatenate([blk, jnp.zeros((128-kw, nw), F32)], axis=0)
                    if nw < 128: blk = jnp.concatenate([blk, jnp.zeros((128, 128-nw), F32)], axis=1)
                    t32[c, j*128:(j+1)*128, :] = blk.T
                for p in range(3):
                    for d in range(DH):
                        rows = t32[c, pl.ds(p * D + d, H, stride=DH), :]
                        r0 = dest(p, d)
                        wqt[r0:r0+H, c*128:(c+1)*128] = rows.astype(BF16)
                if c == DMAC:
                    for f in range(NF):
                        cp_g(f).start(); cp_u(f).start(); cp_d(f).start()
                    for b in range(2, NB): cp_x(b).start()

        def prep_wo():
            cp_o().wait()
            for c in range(5):
                nw = 128 if c < 4 else 64
                blk = woraw[:, c*128:c*128+nw].astype(F32)
                if nw < 128: blk = jnp.concatenate([blk, jnp.zeros((D, 128-nw), F32)], axis=1)
                t32[c, 0:D, :] = blk
            for c in range(5):
                parts = [t32[c, pl.ds(d, H, stride=DH), :] for d in range(DH)] + [jnp.zeros((64, 128), F32)]
                wp = jnp.concatenate(parts, axis=0)
                res = wp.T.astype(BF16)
                nw = 128 if c < 4 else 64
                wot[c*128:c*128+nw, :] = res[:nw]

        dz = jnp.minimum(s, 0)

        def ln_to(dst, first, p):
            for c0 in range(0, TM, LNC):
                x = first(c0)
                m = jnp.sum(x, axis=0, keepdims=True) * (1.0 / D)
                if 'reload' in ablate:
                    x = xs[p, :, pl.ds(pl.multiple_of(c0 + dz * 128, 128), LNC)]
                xc = x - m
                v = jnp.sum(xc * xc, axis=0, keepdims=True) * (1.0 / D)
                r = lax.rsqrt(v + 1e-5)
                if 'reload' in ablate:
                    x = xs[p, :, pl.ds(pl.multiple_of(c0 + dz * 256, 128), LNC)]
                    xc = x - m
                dst[c0:c0+LNC, 0:D] = (xc * r).astype(BF16).T

        def ln_a(pa, xin, use_in, dst):
            def first(c0):
                if use_in is True:
                    x = xin[:, c0:c0+LNC].astype(F32)
                else:
                    x = jnp.where(use_in, xin[:, c0:c0+LNC].astype(F32), xs[pa, :, c0:c0+LNC])
                xs[pa, :, c0:c0+LNC] = x
                return x
            ln_to(dst, first, pa)

        def ln_blocks(get, dst7, dst_tail):
            def norm(c0):
                x = get(c0)
                m = jnp.sum(x, axis=0, keepdims=True) * (1.0 / D)
                xc = x - m
                v = jnp.sum(xc * xc, axis=0, keepdims=True) * (1.0 / D)
                return xc * lax.rsqrt(v + 1e-5)
            for c0 in range(0, HT, LNC):
                n1 = norm(c0); n2 = norm(HT + c0)
                a11 = n1[0:256]; a12 = n1[256:512]; a21 = n2[0:256]; a22 = n2[256:512]
                for j, val in enumerate([a11 + a22, a21 + a22, a11, a22, a11 + a12, a21 - a11, a12 - a22]):
                    dst7[j, rs(c0, LNC), :] = pk(val.astype(BF16).T)
                dst_tail[c0:c0+LNC, 0:64] = n1[512:576].astype(BF16).T
                dst_tail[HT+c0:HT+c0+LNC, 0:64] = n2[512:576].astype(BF16).T

        def ln_f(pf):
            ln_blocks(lambda c0: xs[pf, :, c0:c0+LNC], sa, xnf)

        def ln_a2(pa, xin, use_in, dst7, dst_tail):
            def first(c0):
                if use_in is True:
                    x = xin[:, c0:c0+LNC].astype(F32)
                else:
                    x = jnp.where(use_in, xin[:, c0:c0+LNC].astype(F32), xs[pa, :, c0:c0+LNC])
                xs[pa, :, c0:c0+LNC] = x
                return x
            ln_blocks(first, dst7, dst_tail)

        def qkv_prep():
            NH = 896
            for r in range(0, NH, PRB):
                r1 = slice(r, r + PRB); r2 = slice(NH + r, NH + r + PRB)
                b11 = wqt[r1, 0:256].astype(F32); b12 = wqt[r2, 0:256].astype(F32)
                b21 = wqt[r1, 256:512].astype(F32); b22 = wqt[r2, 256:512].astype(F32)
                for j, val in enumerate([b11 + b22, b12 - b22, b21 - b11, b11 + b12, b21 + b22]):
                    tq[j, rs(r, PRB), :] = pk(val.astype(BF16))

        def qkv_matmul(src7, src_tail):
            NH = 896
            m1 = dnt(upk(src7[0]), upk(tq[0]))
            m2 = dnt(upk(src7[1]), wqt[0:NH, 0:256])
            m3 = dnt(upk(src7[2]), upk(tq[1]))
            m4 = dnt(upk(src7[3]), upk(tq[2]))
            m5 = dnt(upk(src7[4]), wqt[NH:2*NH, 256:512])
            m6 = dnt(upk(src7[5]), upk(tq[3]))
            m7 = dnt(upk(src7[6]), upk(tq[4]))
            tl = dnt(src_tail[:, 0:64], wqt[:, 512:576])
            top = jnp.concatenate([m1 + m4 - m5 + m7, m3 + m5], axis=1)
            bot = jnp.concatenate([m2 + m4, m1 - m2 + m3 + m6], axis=1)
            return jnp.concatenate([top, bot], axis=0) + tl

        def wo_stage(pf):
            xs[pf] += lax.dot_general(wot[:, 0:D], os_[:, 0:D], NT, preferred_element_type=F32)

        def qkv_stage(pa, la, src, src_tail=None):
            for c in range(5):
                kb[pa, c, 0:HALO, :] = kt[la, c]
                vb[pa, c, 0:HALO, :] = vt[la, c]
            if QS: qkv = qkv_matmul(src, src_tail)
            else: qkv = lax.dot_general(src[:, 0:D], wqt[:, 0:D], NT, preferred_element_type=F32)
            lane = lax.broadcasted_iota(jnp.int32, (TM, 128), 1)
            qs[pa, :, 0:512] = qkv[:, 0:512] * qscale
            t4 = qkv[:, 512:640]
            qs[pa, :, 512:640] = jnp.where(lane < 64, t4 * qscale, 0.0)
            for c in range(5):
                kk = qkv[:, 640+c*128:640+(c+1)*128] if c < 4 else pltpu.roll(t4, 64, 1)
                vv = qkv[:, 1152+c*128:1152+(c+1)*128]
                kb[pa, c, HALO:HALO+TM, :] = kk
                vb[pa, c, HALO:HALO+TM, :] = vv
                kt[la, c] = kk[TM-HALO:, :]
                vt[la, c] = vv[TM-HALO:, :]

        def first_block_halo(pa):
            for c in range(5):
                kb[pa, c, 0:HALO, :] = jnp.zeros((HALO, 128), F32)
                vb[pa, c, 0:HALO, :] = jnp.broadcast_to(vb[pa, c, HALO:HALO+1, :], (HALO, 128))

        def att_tile(pa, r0, rt, mask_base):
            q = [qs[pa, pl.ds(r0, rt), c*128:(c+1)*128] for c in range(5)]
            lg = []
            for w in range(NW):
                acc = None
                for c in range(5):
                    kk = kb[pa, c, pl.ds(r0 + HALO - DIL*w, rt), :]
                    p = q[c] * kk
                    acc = p if acc is None else acc + p
                acc = acc + pltpu.roll(acc, 64, 1)
                acc = acc + pltpu.roll(acc, 32, 1)
                if mask_base is not None and w > 0:
                    pos = mask_base + lax.broadcasted_iota(jnp.int32, (rt, 128), 0)
                    acc = jnp.where(pos >= DIL*w, acc, -1e9 * LOG2E)
                lg.append(acc)
            mx = lg[0]
            for w in range(1, NW): mx = jnp.maximum(mx, lg[w])
            e = [jnp.exp2(a - mx) for a in lg]
            sm = e[0]
            for w in range(1, NW): sm = sm + e[w]
            inv = 1.0 / sm
            res = []
            for c in range(5):
                acc = None
                for w in range(NW):
                    vv = vb[pa, c, pl.ds(r0 + HALO - DIL*w, rt), :]
                    t = e[w] * vv
                    acc = t if acc is None else acc + t
                o = (acc * inv).astype(BF16)
                os_[pl.ds(r0, rt), c*128:(c+1)*128] = o
                res.append(o)
            return res

        def att_rows(pa, base, n, rt, pos0):
            if 'noatt' in ablate: return
            att_tile(pa, base, HALO, pos0)
            r = HALO
            while r < n:
                t = min(rt, n - r)
                att_tile(pa, base + r, t, None)
                r += t

        def pk(x):
            return pltpu.bitcast(x, jnp.uint32) if U32 else x
        def upk(x):
            return pltpu.bitcast(x, BF16) if U32 else x
        def rs(r0, n):
            return slice(r0 // 2, (r0 + n) // 2) if U32 else slice(r0, r0 + n)
        def ra(n):
            return slice(0, n // 2) if U32 else slice(0, n)

        def dot(a, b): return jnp.dot(a, b, preferred_element_type=F32)
        def dnt(a, b): return lax.dot_general(a, b, NT, preferred_element_type=F32)

        def ffn_prep_gu(f, k1, k2, ko):
            for w, t in ((wg, tg), (wu, tu)):
                for r in range(0, 256, PRB):
                    r1 = slice(r, r + PRB); r2 = slice(256 + r, 256 + r + PRB)
                    b11 = w[f, r1, k1].astype(F32); b12 = w[f, r1, k2].astype(F32)
                    b21 = w[f, r2, k1].astype(F32); b22 = w[f, r2, k2].astype(F32)
                    for j, val in enumerate([b11 + b22, b12 - b22, b21 - b11, b11 + b12, b21 + b22]):
                        t[f, j, rs(r, PRB), ko] = pk(val.astype(BF16))

        def ffn_prep_d(f, k1, k2, ko):
            for r in range(0, 288, PRB):
                n = min(PRB, 288 - r)
                r1 = slice(r, r + n); r2 = slice(288 + r, 288 + r + n)
                a11 = wd[f, r1, k1].astype(F32); a12 = wd[f, r1, k2].astype(F32)
                a21 = wd[f, r2, k1].astype(F32); a22 = wd[f, r2, k2].astype(F32)
                td[f, 0, rs(r, n), ko] = pk((a11 + a22).astype(BF16))
                td[f, 1, rs(r, n), ko] = pk((a21 + a22).astype(BF16))
                td[f, 2, rs(r, n), ko] = pk((a11 + a12).astype(BF16))
                td[f, 3, rs(r, n), ko] = pk((a21 - a11).astype(BF16))
                td[f, 4, rs(r, n), ko] = pk((a12 - a22).astype(BF16))

        def ffn_prep_inline(f):
            cp_g(f).wait(); cp_u(f).wait(); cp_d(f).wait()
            for c in range(FC // 256):
                gi = c // (fs // 128); cc = c % (fs // 128)
                ffn_prep_gu(f, slice(gi * GS + cc * 128, gi * GS + (cc + 1) * 128),
                           slice(gi * GS + fs + cc * 128, gi * GS + fs + (cc + 1) * 128), slice(c * 128, (c + 1) * 128))
                ffn_prep_d(f, slice(gi * GS + cc * 128, gi * GS + (cc + 1) * 128),
                           slice(gi * GS + fs + cc * 128, gi * GS + fs + (cc + 1) * 128), slice(c * 128, (c + 1) * 128))

        def ffn_prep(f):
            def dbody(c, _):
                gi = c // (fs // 128); cc = c % (fs // 128)
                k1 = pl.ds(pl.multiple_of(gi * GS + cc * 128, 128), 128)
                k2 = pl.ds(pl.multiple_of(gi * GS + fs + cc * 128, 128), 128)
                ko = pl.ds(pl.multiple_of(c * 128, 128), 128)
                ffn_prep_d(f, k1, k2, ko)
                q = c // (fs // 256); qq = c % (fs // 256)
                j1 = pl.ds(pl.multiple_of(q * fs + qq * 128, 128), 128)
                j2 = pl.ds(pl.multiple_of(q * fs + fs // 2 + qq * 128, 128), 128)
                ffn_prep_gu(f, j1, j2, ko)
                return 0
            lax.fori_loop(0, FC // 256, dbody, 0)

        def ffn_up(f, gi):
            tl = xnf[:, 0:64]
            hh = fs // 2
            def proj(w, t, kh):
                c0 = gi * GS + kh * fs
                k1 = slice(c0, c0 + hh); k2 = slice(c0 + hh, c0 + fs)
                ko = slice(c0 // 2, c0 // 2 + hh)
                m1 = dot(upk(sa[0]), upk(t[f, 0, :, ko]))
                m2 = dot(upk(sa[1]), w[f, 0:256, k1])
                m3 = dot(upk(sa[2]), upk(t[f, 1, :, ko]))
                m4 = dot(upk(sa[3]), upk(t[f, 2, :, ko]))
                m5 = dot(upk(sa[4]), w[f, 256:512, k2])
                m6 = dot(upk(sa[5]), upk(t[f, 3, :, ko]))
                m7 = dot(upk(sa[6]), upk(t[f, 4, :, ko]))
                tt = dot(tl, w[f, 512:576, c0:c0+fs])
                top = jnp.concatenate([m1 + m4 - m5 + m7, m3 + m5], axis=1) + tt[0:HT]
                bot = jnp.concatenate([m2 + m4, m1 - m2 + m3 + m6], axis=1) + tt[HT:TM]
                return top, bot
            hs = {}
            for kh in range(2):
                g = proj(wg, tg, kh); u = proj(wu, tu, kh)
                hs[(0, kh)] = _gelu(g[0]) * u[0]
                hs[(1, kh)] = _gelu(g[1]) * u[1]
            h11, h12, h21, h22 = hs[(0, 0)], hs[(0, 1)], hs[(1, 0)], hs[(1, 1)]
            b11, b12, b21, b22 = h11, h21, h12, h22
            return [v.astype(BF16) for v in (b11 + b22, b11, b12 - b22, b21 - b11, b22, b11 + b12, b21 + b22)]

        def ffn_down(pf, f, gi, hb):
            ko = slice(gi * fs, (gi + 1) * fs)
            k1 = slice(gi * GS, gi * GS + fs); k2 = slice(gi * GS + fs, (gi + 1) * GS)
            n1 = dnt(upk(td[f, 0, :, ko]), hb[0])
            n2 = dnt(upk(td[f, 1, :, ko]), hb[1])
            n3 = dnt(wd[f, 0:288, k1], hb[2])
            n4 = dnt(wd[f, 288:576, k2], hb[3])
            n5 = dnt(upk(td[f, 2, :, ko]), hb[4])
            n6 = dnt(upk(td[f, 3, :, ko]), hb[5])
            n7 = dnt(upk(td[f, 4, :, ko]), hb[6])
            xs[pf, 0:288, 0:HT] += n1 + n4 - n5 + n7
            xs[pf, 0:288, HT:TM] += n3 + n5
            xs[pf, 288:576, 0:HT] += n2 + n4
            xs[pf, 288:576, HT:TM] += n1 - n2 + n3 + n6

        def ffn_chunk(pf, f, att_parts):
            prev = None
            for gi in range(NG):
                cur = ffn_up(f, gi)
                outs = att_parts[gi]()
                if TIE and outs:
                    z = cur[1][0:RT, 0:128]
                    for o in outs: z = jnp.where(never, o, z)
                    top = jnp.concatenate([z, cur[1][0:RT, 128:]], axis=1) if fs > 128 else z
                    cur[1] = jnp.concatenate([top, cur[1][RT:]], axis=0)
                if prev is not None: ffn_down(pf, f, gi - 1, prev)
                prev = cur
            ffn_down(pf, f, NG - 1, prev)

        @pl.when(s == 0)
        def _():
            flag[0] = 0
        never = flag[0] != 0
        pa = s % 2
        pf = 1 - pa
        la = (s // 2) % 2
        ab = blk_of(s)

        @pl.when(s == 0)
        @jax.named_scope("P0")
        def _():
            prep()
            if QS: qkv_prep()
            cp_x(1).wait()
            if QS:
                qkv_stage(0, 0, sq, xqt)
                ln_a2(1, xin.at[1], True, sa, xnf)
            else:
                qkv_stage(0, 0, xna)
                ln_a(1, xin.at[1], True, xn1)
            first_block_halo(0)
            prep_wo()

        @pl.when(s == 0)
        @jax.named_scope("P1")
        def _():
            if PP >= 1: ffn_prep_inline(0)
            if 'attlast' in ablate:
                (qkv_stage(1, 0, sa, xnf) if QS else qkv_stage(1, 0, xn1))
                att_rows(0, 0, TM, RTP, 0)
            else:
                att_rows(0, 0, TM, RTP, 0)
                (qkv_stage(1, 0, sa, xnf) if QS else qkv_stage(1, 0, xn1))

        for b in range(2, NB):
            @pl.when(s == 2 * b)
            def _():
                cp_x(b).wait()

        @pl.when(jnp.logical_and(s > 1, s < NSLOT - 1))
        @jax.named_scope("R")
        def _():
            if QS: ln_a2(pa, xin.at[jnp.minimum(ab, NB - 1)], la == 0, sq, xqt)
            else: ln_a(pa, xin.at[jnp.minimum(ab, NB - 1)], la == 0, xna)
            wo_stage(pf)
            (qkv_stage(pa, la, sq, xqt) if QS else qkv_stage(pa, la, xna))
            ln_f(pf)

        if PP >= 2:
            @pl.when(s == 1)
            @jax.named_scope("RS1")
            def _():
                ffn_prep_inline(1)
                wo_stage(pf)
                ln_f(pf)

        @pl.when(jnp.logical_or(s == 1, s == NSLOT - 1) if PP < 2 else s == NSLOT - 1)
        @jax.named_scope("RS")
        def _():
            wo_stage(pf)
            ln_f(pf)

        @pl.when(s == 2)
        def _():
            first_block_halo(0)

        @pl.when(s > 0)
        @jax.named_scope("LOOP")
        def _():
            def body(f, _):
                @pl.when(s == 1)
                def _():
                    for ff in range(PP, NF):
                        @pl.when(f == ff)
                        def _():
                            cp_g(ff).wait(); cp_u(ff).wait(); cp_d(ff).wait()
                    @pl.when(f >= PP)
                    def _():
                        ffn_prep(f)
                base = pl.multiple_of(jnp.minimum(f * PR, TM - PR), RT)
                tiles = [functools.partial(att_tile, pa, base + r, RT, (ab * TM + base) if r == 0 else None)
                         for r in range(0, PR, RT)]
                nper = -(-len(tiles) // NG)
                def part(j):
                    def run():
                        if 'noatt' in ablate: return []
                        return [o for t in tiles[j*nper:(j+1)*nper] for o in t()]
                    return run
                ffn_chunk(pf, f, [part(j) for j in range(NG)])
                return 0
            lax.fori_loop(0, NF, body, 0)

        @pl.when(jnp.logical_and(s > 0, ((s - 1) // 2) % 2 == 1))
        def _():
            o_ref[...] = xs[pf].astype(o_ref.dtype)

    def x_map(s):
        la = (s // 2) % 2
        b = jnp.where(la == 0, blk_of(s), 2 * (s // 4) + 1)
        return (0, jnp.clip(b, 0, NB - 1))

    def o_map(s):
        fidx = jnp.maximum(s - 1, 0)
        b = 2 * (fidx // 4) + jnp.where(fidx % 4 == 3, 1, 0)
        return (0, b)

    def fn(A_x, A_wqkv, A_wo, B_x, B_w_gate, B_w_up, B_w_down):
        xT = A_x.reshape(S, D).T
        out = pl.pallas_call(
            kernel,
            grid=(NSLOT,),
            in_specs=[pl.BlockSpec(memory_space=pltpu.HBM)] * 6,
            out_specs=pl.BlockSpec((D, TM), o_map),
            out_shape=jax.ShapeDtypeStruct((D, S), BF16),
            scratch_shapes=[
                pltpu.VMEM((NB, D, TM), BF16), pltpu.VMEM((D, 3 * D), BF16), pltpu.VMEM((D, D), BF16),
                pltpu.VMEM((5, 1792, 128), F32),
                pltpu.VMEM((1792, 640), BF16), pltpu.VMEM((D, 640), BF16),
                pltpu.VMEM((NF, D, FC), BF16), pltpu.VMEM((NF, D, FC), BF16), pltpu.VMEM((NF, D, FC), BF16),
                pltpu.VMEM((NF, 5, 128, FC // 2), jnp.uint32), pltpu.VMEM((NF, 5, 128, FC // 2), jnp.uint32),
                pltpu.VMEM((NF, 5, 144, FC // 2), jnp.uint32) if U32 else pltpu.VMEM((NF, 5, 288, FC // 2), BF16),
                pltpu.VMEM((2, D, TM), F32), pltpu.VMEM((TM, 640), BF16), pltpu.VMEM((TM, 640), BF16), pltpu.VMEM((TM, 128), BF16), pltpu.VMEM((7, HT // 2, 256), jnp.uint32) if U32 else pltpu.VMEM((7, HT, 256), BF16),
                pltpu.VMEM((7, HT // 2, 256), jnp.uint32) if U32 else pltpu.VMEM((7, HT, 256), BF16),
                pltpu.VMEM((TM, 128), BF16),
                pltpu.VMEM((5, 448, 256), jnp.uint32) if U32 else pltpu.VMEM((5, 896, 256), BF16),
                pltpu.VMEM((2, TM, 640), F32),
                pltpu.VMEM((2, 5, TM + HALO + KPAD, 128), F32), pltpu.VMEM((2, 5, TM + HALO + KPAD, 128), F32),
                pltpu.VMEM((2, 5, HALO, 128), F32), pltpu.VMEM((2, 5, HALO, 128), F32),
                pltpu.VMEM((TM, 640), BF16),
                pltpu.SemaphoreType.DMA((2 + 3 * NF,)), pltpu.SemaphoreType.DMA((5 + NB,)), pltpu.SMEM((1,), jnp.int32),
            ],
            compiler_params=pltpu.CompilerParams(dimension_semantics=("arbitrary",), vmem_limit_bytes=112 * 1024 * 1024),
        )(xT, A_wqkv, A_wo, B_w_gate, B_w_up, B_w_down.T)
        return out.T.reshape(1, S, D)
    return fn


_fn = make_kernel(ablate='attlast')


@jax.jit
def pallas_interleave_layers__sliding_local_dilated__glu_gated_geglu__prompt_kernel(
    A_x: jax.Array,
    A_wqkv: jax.Array,
    A_wo: jax.Array,
    B_x: jax.Array,
    B_w_gate: jax.Array,
    B_w_up: jax.Array,
    B_w_down: jax.Array,
):
    return _fn(A_x, A_wqkv, A_wo, B_x, B_w_gate, B_w_up, B_w_down)
```

```python
import functools
import numpy as np
import jax
import jax.numpy as jnp
from jax import lax
import jax.experimental.pallas as pl
import jax.experimental.pallas.tpu as pltpu

S, D, F, H, DH = 2048, 576, 4608, 32, 18
NW, DIL = 8, 2
HALO = 16
LOG2E = 1.4426950408889634
NT = (((1,), (1,)), ((), ()))
F32, BF16 = jnp.float32, jnp.bfloat16

def _ln_t(x):
    m = jnp.sum(x, axis=0, keepdims=True) * (1.0 / D)
    xc = x - m
    v = jnp.sum(xc * xc, axis=0, keepdims=True) * (1.0 / D)
    return (xc * lax.rsqrt(v + 1e-5)).astype(BF16)

def _gelu(g):
    c = np.float32(np.sqrt(2 / np.pi))
    inner = g * (c + (c * 0.044715) * (g * g))
    hg = 0.5 * g
    return hg + hg * jnp.tanh(inner)

def make_kernel(TM=512, FC=1536, GS=512, PRB=32, PP=0, LT=-1, QS=1, TIE=0, U32=1, RT=16, RTP=128, LNC=128, KPAD=16, DMAC=4, XPAD=0, QPAD=0, ablate=''):
    NB = S // TM
    NF = F // FC
    NSLOT = 2 * NB + 1
    PR = -(-TM // NF // RT) * RT
    HT = TM // 2
    fs = GS // 2
    NG = FC // GS

    def blk_of(a):
        return 2 * (a // 4) + a % 2

    def kernel(x_hbm, wqkv_hbm, wo_hbm, wg_hbm, wu_hbm, wd_hbm, o_ref,
               xin, wraw, woraw, t32, wqt, wot, wg, wu, wd, tg, tu, td, xs, xna, xn1, xnf, sa, sq, xqt, tq, qs, kb, vb, kt, vt, os_, sems, sems2, flag):
        s = pl.program_id(0)
        def cp_qkv(c):
            n = 128 if c < 4 else 64
            return pltpu.make_async_copy(wqkv_hbm.at[pl.ds(c*128, n), :], wraw.at[pl.ds(c*128, n), :], sems2.at[c])
        def cp_x(b): return pltpu.make_async_copy(x_hbm.at[:, pl.ds(b*TM, TM)], xin.at[b], sems2.at[5+b])
        def cp_o(): return pltpu.make_async_copy(wo_hbm, woraw, sems.at[1])
        def cp_g(f): return pltpu.make_async_copy(wg_hbm.at[:, pl.ds(f*FC, FC)], wg.at[f], sems.at[2+3*f])
        def cp_u(f): return pltpu.make_async_copy(wu_hbm.at[:, pl.ds(f*FC, FC)], wu.at[f], sems.at[3+3*f])
        def cp_d(f): return pltpu.make_async_copy(wd_hbm.at[:, pl.ds(f*FC, FC)], wd.at[f], sems.at[4+3*f])

        qscale = (DH ** -0.5) * LOG2E

        def prep():
            cp_x(0).start()
            for c in range(5): cp_qkv(c).start()
            cp_x(1).start(); cp_o().start()
            kt[...] = jnp.zeros(kt.shape, F32)
            vt[...] = jnp.zeros(vt.shape, F32)
            wqt[1728:1792, :] = jnp.zeros((64, 640), BF16)
            cp_x(0).wait()
            (ln_a2(0, xin.at[0], True, sq, xqt) if QS else ln_a(0, xin.at[0], True, xna))
            def dest(p, d):
                if p == 0: return d * 32
                if p == 1: return 576 + (d - 16) * 32 if d >= 16 else 640 + d * 32
                return 1152 + d * 32
            for c in range(5):
                cp_qkv(c).wait()
                kw = 128 if c < 4 else 64
                for j in range(14):
                    nw = 128 if j < 13 else 64
                    blk = wraw[c*128:c*128+kw, j*128:j*128+nw].astype(F32)
                    if kw < 128: blk = jnp.concatenate([blk, jnp.zeros((128-kw, nw), F32)], axis=0)
                    if nw < 128: blk = jnp.concatenate([blk, jnp.zeros((128, 128-nw), F32)], axis=1)
                    t32[c, j*128:(j+1)*128, :] = blk.T
                for p in range(3):
                    for d in range(DH):
                        rows = t32[c, pl.ds(p * D + d, H, stride=DH), :]
                        r0 = dest(p, d)
                        wqt[r0:r0+H, c*128:(c+1)*128] = rows.astype(BF16)
                if c == DMAC:
                    for f in range(NF):
                        cp_g(f).start(); cp_u(f).start(); cp_d(f).start()
                    for b in range(2, NB): cp_x(b).start()

        def prep_wo():
            cp_o().wait()
            for c in range(5):
                nw = 128 if c < 4 else 64
                blk = woraw[:, c*128:c*128+nw].astype(F32)
                if nw < 128: blk = jnp.concatenate([blk, jnp.zeros((D, 128-nw), F32)], axis=1)
                t32[c, 0:D, :] = blk
            for c in range(5):
                parts = [t32[c, pl.ds(d, H, stride=DH), :] for d in range(DH)] + [jnp.zeros((64, 128), F32)]
                wp = jnp.concatenate(parts, axis=0)
                res = wp.T.astype(BF16)
                nw = 128 if c < 4 else 64
                wot[c*128:c*128+nw, :] = res[:nw]

        dz = jnp.minimum(s, 0)

        def ln_to(dst, first, p):
            for c0 in range(0, TM, LNC):
                x = first(c0)
                m = jnp.sum(x, axis=0, keepdims=True) * (1.0 / D)
                if 'reload' in ablate:
                    x = xs[p, :, pl.ds(pl.multiple_of(c0 + dz * 128, 128), LNC)]
                xc = x - m
                v = jnp.sum(xc * xc, axis=0, keepdims=True) * (1.0 / D)
                r = lax.rsqrt(v + 1e-5)
                if 'reload' in ablate:
                    x = xs[p, :, pl.ds(pl.multiple_of(c0 + dz * 256, 128), LNC)]
                    xc = x - m
                dst[c0:c0+LNC, 0:D] = (xc * r).astype(BF16).T

        def ln_a(pa, xin, use_in, dst):
            def first(c0):
                if use_in is True:
                    x = xin[:, c0:c0+LNC].astype(F32)
                else:
                    x = jnp.where(use_in, xin[:, c0:c0+LNC].astype(F32), xs[pa, :, c0:c0+LNC])
                xs[pa, :, c0:c0+LNC] = x
                return x
            ln_to(dst, first, pa)

        def ln_blocks(get, dst7, dst_tail):
            def norm(c0):
                x = get(c0)
                m = jnp.sum(x, axis=0, keepdims=True) * (1.0 / D)
                xc = x - m
                v = jnp.sum(xc * xc, axis=0, keepdims=True) * (1.0 / D)
                return xc * lax.rsqrt(v + 1e-5)
            for c0 in range(0, HT, LNC):
                n1 = norm(c0); n2 = norm(HT + c0)
                a11 = n1[0:256]; a12 = n1[256:512]; a21 = n2[0:256]; a22 = n2[256:512]
                for j, val in enumerate([a11 + a22, a21 + a22, a11, a22, a11 + a12, a21 - a11, a12 - a22]):
                    dst7[j, rs(c0, LNC), :] = pk(val.astype(BF16).T)
                dst_tail[c0:c0+LNC, 0:64] = n1[512:576].astype(BF16).T
                dst_tail[HT+c0:HT+c0+LNC, 0:64] = n2[512:576].astype(BF16).T

        def ln_f(pf, tie=None):
            def get(c0):
                x = xs[pf, :, c0:c0+LNC]
                if tie is not None:
                    x = jnp.concatenate([jnp.where(never, tie, x[0:8]), x[8:]], axis=0)
                return x
            ln_blocks(get, sa, xnf)

        def ln_a2(pa, xin, use_in, dst7, dst_tail):
            def first(c0):
                if use_in is True:
                    x = xin[:, c0:c0+LNC].astype(F32)
                else:
                    x = jnp.where(use_in, xin[:, c0:c0+LNC].astype(F32), xs[pa, :, c0:c0+LNC])
                xs[pa, :, c0:c0+LNC] = x
                return x
            ln_blocks(first, dst7, dst_tail)

        def halves(x):
            w = pltpu.bitcast(x, jnp.uint32)
            return [pltpu.unpack_elementwise(w, index=i, packed_dtype=BF16, unpacked_dtype=F32) for i in range(2)]

        def combos(p11, p12, p21, p22, signs):
            b = [halves(p) for p in (p11, p12, p21, p22)]
            outs = []
            for (i, j, sg) in signs:
                vals = [b[i][e] + b[j][e] if sg > 0 else b[i][e] - b[j][e] for e in range(2)]
                outs.append(pltpu.bitcast(pltpu.pack_elementwise(vals, packed_dtype=BF16), jnp.uint32))
            return outs
        RHS_SUMS = [(0, 3, 1), (1, 3, -1), (2, 0, -1), (0, 1, 1), (2, 3, 1)]
        LHS_SUMS = [(0, 3, 1), (2, 3, 1), (0, 1, 1), (2, 0, -1), (1, 3, -1)]

        def qkv_prep():
            NH = 896
            for r in range(0, NH, PRB):
                r1 = slice(r, r + PRB); r2 = slice(NH + r, NH + r + PRB)
                outs = combos(wqt[r1, 0:256], wqt[r2, 0:256], wqt[r1, 256:512], wqt[r2, 256:512], RHS_SUMS)
                for j, val in enumerate(outs):
                    tq[j, rs(r, PRB), :] = val

        def qkv_matmul(src7, src_tail):
            NH = 896
            m1 = dnt(upk(src7[0]), upk(tq[0]))
            m2 = dnt(upk(src7[1]), wqt[0:NH, 0:256])
            m3 = dnt(upk(src7[2]), upk(tq[1]))
            m4 = dnt(upk(src7[3]), upk(tq[2]))
            m5 = dnt(upk(src7[4]), wqt[NH:2*NH, 256:512])
            m6 = dnt(upk(src7[5]), upk(tq[3]))
            m7 = dnt(upk(src7[6]), upk(tq[4]))
            tl = dnt(src_tail[:, 0:64], wqt[:, 512:576])
            top = jnp.concatenate([m1 + m4 - m5 + m7, m3 + m5], axis=1)
            bot = jnp.concatenate([m2 + m4, m1 - m2 + m3 + m6], axis=1)
            return jnp.concatenate([top, bot], axis=0) + tl, [m1, m2, m3, m4, m5, m6, m7, tl][LT][0:8, 0:LNC]

        def wo_stage(pf):
            xs[pf] += lax.dot_general(wot[:, 0:D], os_[:, 0:D], NT, preferred_element_type=F32)

        def qkv_stage(pa, la, src, src_tail=None):
            for c in range(5):
                kb[pa, c, 0:HALO, :] = kt[la, c]
                vb[pa, c, 0:HALO, :] = vt[la, c]
            tie = None
            if QS: qkv, tie = qkv_matmul(src, src_tail)
            else: qkv = lax.dot_general(src[:, 0:D], wqt[:, 0:D], NT, preferred_element_type=F32)
            lane = lax.broadcasted_iota(jnp.int32, (TM, 128), 1)
            qs[pa, :, 0:512] = qkv[:, 0:512] * qscale
            t4 = qkv[:, 512:640]
            qs[pa, :, 512:640] = jnp.where(lane < 64, t4 * qscale, 0.0)
            for c in range(5):
                kk = qkv[:, 640+c*128:640+(c+1)*128] if c < 4 else pltpu.roll(t4, 64, 1)
                vv = qkv[:, 1152+c*128:1152+(c+1)*128]
                kb[pa, c, HALO:HALO+TM, :] = kk
                vb[pa, c, HALO:HALO+TM, :] = vv
                kt[la, c] = kk[TM-HALO:, :]
                vt[la, c] = vv[TM-HALO:, :]
            return tie

        def first_block_halo(pa):
            for c in range(5):
                kb[pa, c, 0:HALO, :] = jnp.zeros((HALO, 128), F32)
                vb[pa, c, 0:HALO, :] = jnp.broadcast_to(vb[pa, c, HALO:HALO+1, :], (HALO, 128))

        def att_tile(pa, r0, rt, mask_base):
            q = [qs[pa, pl.ds(r0, rt), c*128:(c+1)*128] for c in range(5)]
            lg = []
            for w in range(NW):
                acc = None
                for c in range(5):
                    kk = kb[pa, c, pl.ds(r0 + HALO - DIL*w, rt), :]
                    p = q[c] * kk
                    acc = p if acc is None else acc + p
                acc = acc + pltpu.roll(acc, 64, 1)
                acc = acc + pltpu.roll(acc, 32, 1)
                if mask_base is not None and w > 0:
                    pos = mask_base + lax.broadcasted_iota(jnp.int32, (rt, 128), 0)
                    acc = jnp.where(pos >= DIL*w, acc, -1e9 * LOG2E)
                lg.append(acc)
            mx = lg[0]
            for w in range(1, NW): mx = jnp.maximum(mx, lg[w])
            e = [jnp.exp2(a - mx) for a in lg]
            sm = e[0]
            for w in range(1, NW): sm = sm + e[w]
            inv = 1.0 / sm
            res = []
            for c in range(5):
                acc = None
                for w in range(NW):
                    vv = vb[pa, c, pl.ds(r0 + HALO - DIL*w, rt), :]
                    t = e[w] * vv
                    acc = t if acc is None else acc + t
                o = (acc * inv).astype(BF16)
                os_[pl.ds(r0, rt), c*128:(c+1)*128] = o
                res.append(o)
            return res

        def att_rows(pa, base, n, rt, pos0):
            if 'noatt' in ablate: return
            att_tile(pa, base, HALO, pos0)
            r = HALO
            while r < n:
                t = min(rt, n - r)
                att_tile(pa, base + r, t, None)
                r += t

        def pk(x):
            return pltpu.bitcast(x, jnp.uint32) if U32 else x
        def upk(x):
            return pltpu.bitcast(x, BF16) if U32 else x
        def rs(r0, n):
            return slice(r0 // 2, (r0 + n) // 2) if U32 else slice(r0, r0 + n)
        def ra(n):
            return slice(0, n // 2) if U32 else slice(0, n)

        def dot(a, b): return jnp.dot(a, b, preferred_element_type=F32)
        def dnt(a, b): return lax.dot_general(a, b, NT, preferred_element_type=F32)

        def ffn_prep_gu(f, k1, k2, ko):
            for w, t in ((wg, tg), (wu, tu)):
                for r in range(0, 256, PRB):
                    r1 = slice(r, r + PRB); r2 = slice(256 + r, 256 + r + PRB)
                    outs = combos(w[f, r1, k1], w[f, r1, k2], w[f, r2, k1], w[f, r2, k2], RHS_SUMS)
                    for j, val in enumerate(outs):
                        t[f, j, rs(r, PRB), ko] = val

        def ffn_prep_d(f, k1, k2, ko):
            for r in range(0, 288, PRB):
                n = min(PRB, 288 - r)
                r1 = slice(r, r + n); r2 = slice(288 + r, 288 + r + n)
                outs = combos(wd[f, r1, k1], wd[f, r1, k2], wd[f, r2, k1], wd[f, r2, k2], LHS_SUMS)
                for j, val in enumerate(outs):
                    td[f, j, rs(r, n), ko] = val

        def ffn_prep_inline(f):
            cp_g(f).wait(); cp_u(f).wait(); cp_d(f).wait()
            for c in range(FC // 256):
                gi = c // (fs // 128); cc = c % (fs // 128)
                ffn_prep_gu(f, slice(gi * GS + cc * 128, gi * GS + (cc + 1) * 128),
                           slice(gi * GS + fs + cc * 128, gi * GS + fs + (cc + 1) * 128), slice(c * 128, (c + 1) * 128))
                ffn_prep_d(f, slice(gi * GS + cc * 128, gi * GS + (cc + 1) * 128),
                           slice(gi * GS + fs + cc * 128, gi * GS + fs + (cc + 1) * 128), slice(c * 128, (c + 1) * 128))

        def ffn_prep(f):
            def dbody(c, _):
                gi = c // (fs // 128); cc = c % (fs // 128)
                k1 = pl.ds(pl.multiple_of(gi * GS + cc * 128, 128), 128)
                k2 = pl.ds(pl.multiple_of(gi * GS + fs + cc * 128, 128), 128)
                ko = pl.ds(pl.multiple_of(c * 128, 128), 128)
                ffn_prep_d(f, k1, k2, ko)
                q = c // (fs // 256); qq = c % (fs // 256)
                j1 = pl.ds(pl.multiple_of(q * fs + qq * 128, 128), 128)
                j2 = pl.ds(pl.multiple_of(q * fs + fs // 2 + qq * 128, 128), 128)
                ffn_prep_gu(f, j1, j2, ko)
                return 0
            lax.fori_loop(0, FC // 256, dbody, 0)

        def ffn_up(f, gi):
            tl = xnf[:, 0:64]
            hh = fs // 2
            def proj(w, t, kh):
                c0 = gi * GS + kh * fs
                k1 = slice(c0, c0 + hh); k2 = slice(c0 + hh, c0 + fs)
                ko = slice(c0 // 2, c0 // 2 + hh)
                m1 = dot(upk(sa[0]), upk(t[f, 0, :, ko]))
                m2 = dot(upk(sa[1]), w[f, 0:256, k1])
                m3 = dot(upk(sa[2]), upk(t[f, 1, :, ko]))
                m4 = dot(upk(sa[3]), upk(t[f, 2, :, ko]))
                m5 = dot(upk(sa[4]), w[f, 256:512, k2])
                m6 = dot(upk(sa[5]), upk(t[f, 3, :, ko]))
                m7 = dot(upk(sa[6]), upk(t[f, 4, :, ko]))
                tt = dot(tl, w[f, 512:576, c0:c0+fs])
                top = jnp.concatenate([m1 + m4 - m5 + m7, m3 + m5], axis=1) + tt[0:HT]
                bot = jnp.concatenate([m2 + m4, m1 - m2 + m3 + m6], axis=1) + tt[HT:TM]
                return top, bot
            hs = {}
            for kh in range(2):
                g = proj(wg, tg, kh); u = proj(wu, tu, kh)
                hs[(0, kh)] = _gelu(g[0]) * u[0]
                hs[(1, kh)] = _gelu(g[1]) * u[1]
            h11, h12, h21, h22 = hs[(0, 0)], hs[(0, 1)], hs[(1, 0)], hs[(1, 1)]
            b11, b12, b21, b22 = h11, h21, h12, h22
            return [v.astype(BF16) for v in (b11 + b22, b11, b12 - b22, b21 - b11, b22, b11 + b12, b21 + b22)]

        def ffn_down(pf, f, gi, hb):
            ko = slice(gi * fs, (gi + 1) * fs)
            k1 = slice(gi * GS, gi * GS + fs); k2 = slice(gi * GS + fs, (gi + 1) * GS)
            n1 = dnt(upk(td[f, 0, :, ko]), hb[0])
            n2 = dnt(upk(td[f, 1, :, ko]), hb[1])
            n3 = dnt(wd[f, 0:288, k1], hb[2])
            n4 = dnt(wd[f, 288:576, k2], hb[3])
            n5 = dnt(upk(td[f, 2, :, ko]), hb[4])
            n6 = dnt(upk(td[f, 3, :, ko]), hb[5])
            n7 = dnt(upk(td[f, 4, :, ko]), hb[6])
            xs[pf, 0:288, 0:HT] += n1 + n4 - n5 + n7
            xs[pf, 0:288, HT:TM] += n3 + n5
            xs[pf, 288:576, 0:HT] += n2 + n4
            xs[pf, 288:576, HT:TM] += n1 - n2 + n3 + n6

        def ffn_chunk(pf, f, att_parts):
            prev = None
            for gi in range(NG):
                cur = ffn_up(f, gi)
                outs = att_parts[gi]()
                if TIE and outs:
                    z = cur[1][0:RT, 0:128]
                    for o in outs: z = jnp.where(never, o, z)
                    top = jnp.concatenate([z, cur[1][0:RT, 128:]], axis=1) if fs > 128 else z
                    cur[1] = jnp.concatenate([top, cur[1][RT:]], axis=0)
                if prev is not None: ffn_down(pf, f, gi - 1, prev)
                prev = cur
            ffn_down(pf, f, NG - 1, prev)

        @pl.when(s == 0)
        def _():
            flag[0] = 0
        never = flag[0] != 0
        pa = s % 2
        pf = 1 - pa
        la = (s // 2) % 2
        ab = blk_of(s)

        @pl.when(s == 0)
        @jax.named_scope("P0")
        def _():
            prep()
            if QS: qkv_prep()
            cp_x(1).wait()
            if QS:
                qkv_stage(0, 0, sq, xqt)
                ln_a2(1, xin.at[1], True, sa, xnf)
            else:
                qkv_stage(0, 0, xna)
                ln_a(1, xin.at[1], True, xn1)
            first_block_halo(0)
            prep_wo()

        @pl.when(s == 0)
        @jax.named_scope("P1")
        def _():
            if PP >= 1: ffn_prep_inline(0)
            if 'attlast' in ablate:
                (qkv_stage(1, 0, sa, xnf) if QS else qkv_stage(1, 0, xn1))
                att_rows(0, 0, TM, RTP, 0)
            else:
                att_rows(0, 0, TM, RTP, 0)
                (qkv_stage(1, 0, sa, xnf) if QS else qkv_stage(1, 0, xn1))

        for b in range(2, NB):
            @pl.when(s == 2 * b)
            def _():
                cp_x(b).wait()

        @pl.when(jnp.logical_and(s > 1, s < NSLOT - 1))
        @jax.named_scope("R")
        def _():
            if QS: ln_a2(pa, xin.at[jnp.minimum(ab, NB - 1)], la == 0, sq, xqt)
            else: ln_a(pa, xin.at[jnp.minimum(ab, NB - 1)], la == 0, xna)
            wo_stage(pf)
            tie = (qkv_stage(pa, la, sq, xqt) if QS else qkv_stage(pa, la, xna))
            ln_f(pf, tie if LT >= 0 else None)

        if PP >= 2:
            @pl.when(s == 1)
            @jax.named_scope("RS1")
            def _():
                ffn_prep_inline(1)
                wo_stage(pf)
                ln_f(pf)

        @pl.when(jnp.logical_or(s == 1, s == NSLOT - 1) if PP < 2 else s == NSLOT - 1)
        @jax.named_scope("RS")
        def _():
            wo_stage(pf)
            ln_f(pf)

        @pl.when(s == 2)
        def _():
            first_block_halo(0)

        @pl.when(s > 0)
        @jax.named_scope("LOOP")
        def _():
            def body(f, _):
                @pl.when(s == 1)
                def _():
                    for ff in range(PP, NF):
                        @pl.when(f == ff)
                        def _():
                            cp_g(ff).wait(); cp_u(ff).wait(); cp_d(ff).wait()
                    @pl.when(f >= PP)
                    def _():
                        ffn_prep(f)
                base = pl.multiple_of(jnp.minimum(f * PR, TM - PR), RT)
                tiles = [functools.partial(att_tile, pa, base + r, RT, (ab * TM + base) if r == 0 else None)
                         for r in range(0, PR, RT)]
                nper = -(-len(tiles) // NG)
                def part(j):
                    def run():
                        if 'noatt' in ablate: return []
                        return [o for t in tiles[j*nper:(j+1)*nper] for o in t()]
                    return run
                ffn_chunk(pf, f, [part(j) for j in range(NG)])
                return 0
            lax.fori_loop(0, NF, body, 0)

        @pl.when(jnp.logical_and(s > 0, ((s - 1) // 2) % 2 == 1))
        def _():
            o_ref[...] = xs[pf].astype(o_ref.dtype)

    def x_map(s):
        la = (s // 2) % 2
        b = jnp.where(la == 0, blk_of(s), 2 * (s // 4) + 1)
        return (0, jnp.clip(b, 0, NB - 1))

    def o_map(s):
        fidx = jnp.maximum(s - 1, 0)
        b = 2 * (fidx // 4) + jnp.where(fidx % 4 == 3, 1, 0)
        return (0, b)

    def fn(A_x, A_wqkv, A_wo, B_x, B_w_gate, B_w_up, B_w_down):
        xT = A_x.reshape(S, D).T
        out = pl.pallas_call(
            kernel,
            grid=(NSLOT,),
            in_specs=[pl.BlockSpec(memory_space=pltpu.HBM)] * 6,
            out_specs=pl.BlockSpec((D, TM), o_map),
            out_shape=jax.ShapeDtypeStruct((D, S), BF16),
            scratch_shapes=[
                pltpu.VMEM((NB, D, TM), BF16), pltpu.VMEM((D, 3 * D), BF16), pltpu.VMEM((D, D), BF16),
                pltpu.VMEM((5, 1792, 128), F32),
                pltpu.VMEM((1792, 640), BF16), pltpu.VMEM((D, 640), BF16),
                pltpu.VMEM((NF, D, FC), BF16), pltpu.VMEM((NF, D, FC), BF16), pltpu.VMEM((NF, D, FC), BF16),
                pltpu.VMEM((NF, 5, 128, FC // 2), jnp.uint32), pltpu.VMEM((NF, 5, 128, FC // 2), jnp.uint32),
                pltpu.VMEM((NF, 5, 144, FC // 2), jnp.uint32) if U32 else pltpu.VMEM((NF, 5, 288, FC // 2), BF16),
                pltpu.VMEM((2, D, TM), F32), pltpu.VMEM((TM, 640), BF16), pltpu.VMEM((TM, 640), BF16), pltpu.VMEM((TM, 128), BF16), pltpu.VMEM((7, HT // 2, 256), jnp.uint32) if U32 else pltpu.VMEM((7, HT, 256), BF16),
                pltpu.VMEM((7, HT // 2, 256), jnp.uint32) if U32 else pltpu.VMEM((7, HT, 256), BF16),
                pltpu.VMEM((TM, 128), BF16),
                pltpu.VMEM((5, 448, 256), jnp.uint32) if U32 else pltpu.VMEM((5, 896, 256), BF16),
                pltpu.VMEM((2, TM, 640), F32),
                pltpu.VMEM((2, 5, TM + HALO + KPAD, 128), F32), pltpu.VMEM((2, 5, TM + HALO + KPAD, 128), F32),
                pltpu.VMEM((2, 5, HALO, 128), F32), pltpu.VMEM((2, 5, HALO, 128), F32),
                pltpu.VMEM((TM, 640), BF16),
                pltpu.SemaphoreType.DMA((2 + 3 * NF,)), pltpu.SemaphoreType.DMA((5 + NB,)), pltpu.SMEM((1,), jnp.int32),
            ],
            compiler_params=pltpu.CompilerParams(dimension_semantics=("arbitrary",), vmem_limit_bytes=112 * 1024 * 1024),
        )(xT, A_wqkv, A_wo, B_w_gate, B_w_up, B_w_down.T)
        return out.T.reshape(1, S, D)
    return fn


_fn = make_kernel(ablate='attlast')


@jax.jit
def pallas_interleave_layers__sliding_local_dilated__glu_gated_geglu__prompt_kernel(
    A_x: jax.Array,
    A_wqkv: jax.Array,
    A_wo: jax.Array,
    B_x: jax.Array,
    B_w_gate: jax.Array,
    B_w_up: jax.Array,
    B_w_down: jax.Array,
):
    return _fn(A_x, A_wqkv, A_wo, B_x, B_w_gate, B_w_up, B_w_down)
```

```python
import functools
import numpy as np
import jax
import jax.numpy as jnp
from jax import lax
import jax.experimental.pallas as pl
import jax.experimental.pallas.tpu as pltpu

S, D, F, H, DH = 2048, 576, 4608, 32, 18
NW, DIL = 8, 2
HALO = 16
LOG2E = 1.4426950408889634
NT = (((1,), (1,)), ((), ()))
F32, BF16 = jnp.float32, jnp.bfloat16

def _ln_t(x):
    m = jnp.sum(x, axis=0, keepdims=True) * (1.0 / D)
    xc = x - m
    v = jnp.sum(xc * xc, axis=0, keepdims=True) * (1.0 / D)
    return (xc * lax.rsqrt(v + 1e-5)).astype(BF16)

def _gelu(g):
    c = np.float32(np.sqrt(2 / np.pi))
    inner = g * (c + (c * 0.044715) * (g * g))
    hg = 0.5 * g
    return hg + hg * jnp.tanh(inner)

def make_kernel(TM=512, FC=1536, GS=512, PRB=32, PP=0, LT=-1, FLAG='XLA_TPU_EVENLY_DISTRIBUTE_CRITICAL_NODES', QS=1, TIE=0, U32=1, RT=32, PRQ=32, RTP=128, LNC=256, KPAD=16, DMAC=4, XPAD=0, QPAD=0, ablate=''):
    NB = S // TM
    NF = F // FC
    NSLOT = 2 * NB + 1
    PR = -(-TM // NF // PRQ) * PRQ
    HT = TM // 2
    fs = GS // 2
    NG = FC // GS

    def blk_of(a):
        return 2 * (a // 4) + a % 2

    def kernel(x_hbm, wqkv_hbm, wo_hbm, wg_hbm, wu_hbm, wd_hbm, o_ref,
               xin, wraw, woraw, t32, wqt, wot, wg, wu, wd, tg, tu, td, xs, xna, xn1, xnf, sa, sq, xqt, tq, qs, kb, vb, kt, vt, os_, sems, sems2, flag):
        s = pl.program_id(0)
        def cp_qkv(c):
            n = 128 if c < 4 else 64
            return pltpu.make_async_copy(wqkv_hbm.at[pl.ds(c*128, n), :], wraw.at[pl.ds(c*128, n), :], sems2.at[c])
        def cp_x(b): return pltpu.make_async_copy(x_hbm.at[:, pl.ds(b*TM, TM)], xin.at[b], sems2.at[5+b])
        def cp_o(): return pltpu.make_async_copy(wo_hbm, woraw, sems.at[1])
        def cp_g(f): return pltpu.make_async_copy(wg_hbm.at[:, pl.ds(f*FC, FC)], wg.at[f], sems.at[2+3*f])
        def cp_u(f): return pltpu.make_async_copy(wu_hbm.at[:, pl.ds(f*FC, FC)], wu.at[f], sems.at[3+3*f])
        def cp_d(f): return pltpu.make_async_copy(wd_hbm.at[:, pl.ds(f*FC, FC)], wd.at[f], sems.at[4+3*f])

        qscale = (DH ** -0.5) * LOG2E

        def prep():
            cp_x(0).start()
            for c in range(5): cp_qkv(c).start()
            cp_x(1).start(); cp_o().start()
            kt[...] = jnp.zeros(kt.shape, F32)
            vt[...] = jnp.zeros(vt.shape, F32)
            wqt[1728:1792, :] = jnp.zeros((64, 640), BF16)
            cp_x(0).wait()
            (ln_a2(0, xin.at[0], True, sq, xqt) if QS else ln_a(0, xin.at[0], True, xna))
            def dest(p, d):
                if p == 0: return d * 32
                if p == 1: return 576 + (d - 16) * 32 if d >= 16 else 640 + d * 32
                return 1152 + d * 32
            for c in range(5):
                cp_qkv(c).wait()
                kw = 128 if c < 4 else 64
                for j in range(14):
                    nw = 128 if j < 13 else 64
                    blk = wraw[c*128:c*128+kw, j*128:j*128+nw].astype(F32)
                    if kw < 128: blk = jnp.concatenate([blk, jnp.zeros((128-kw, nw), F32)], axis=0)
                    if nw < 128: blk = jnp.concatenate([blk, jnp.zeros((128, 128-nw), F32)], axis=1)
                    t32[c, j*128:(j+1)*128, :] = blk.T
                for p in range(3):
                    for d in range(DH):
                        rows = t32[c, pl.ds(p * D + d, H, stride=DH), :]
                        r0 = dest(p, d)
                        wqt[r0:r0+H, c*128:(c+1)*128] = rows.astype(BF16)
                if c == 4: cp_x(1).wait()
                if c == DMAC:
                    for f in range(NF):
                        cp_g(f).start(); cp_u(f).start(); cp_d(f).start()
                    for b in range(2, NB): cp_x(b).start()

        def prep_wo():
            cp_o().wait()
            for c in range(5):
                nw = 128 if c < 4 else 64
                blk = woraw[:, c*128:c*128+nw].astype(F32)
                if nw < 128: blk = jnp.concatenate([blk, jnp.zeros((D, 128-nw), F32)], axis=1)
                t32[c, 0:D, :] = blk
            for c in range(5):
                parts = [t32[c, pl.ds(d, H, stride=DH), :] for d in range(DH)] + [jnp.zeros((64, 128), F32)]
                wp = jnp.concatenate(parts, axis=0)
                res = wp.T.astype(BF16)
                nw = 128 if c < 4 else 64
                wot[c*128:c*128+nw, :] = res[:nw]

        dz = jnp.minimum(s, 0)

        def ln_to(dst, first, p):
            for c0 in range(0, TM, LNC):
                x = first(c0)
                m = jnp.sum(x, axis=0, keepdims=True) * (1.0 / D)
                if 'reload' in ablate:
                    x = xs[p, :, pl.ds(pl.multiple_of(c0 + dz * 128, 128), LNC)]
                xc = x - m
                v = jnp.sum(xc * xc, axis=0, keepdims=True) * (1.0 / D)
                r = lax.rsqrt(v + 1e-5)
                if 'reload' in ablate:
                    x = xs[p, :, pl.ds(pl.multiple_of(c0 + dz * 256, 128), LNC)]
                    xc = x - m
                dst[c0:c0+LNC, 0:D] = (xc * r).astype(BF16).T

        def ln_a(pa, xin, use_in, dst):
            def first(c0):
                if use_in is True:
                    x = xin[:, c0:c0+LNC].astype(F32)
                else:
                    x = jnp.where(use_in, xin[:, c0:c0+LNC].astype(F32), xs[pa, :, c0:c0+LNC])
                xs[pa, :, c0:c0+LNC] = x
                return x
            ln_to(dst, first, pa)

        def ln_blocks(get, dst7, dst_tail):
            def norm(c0):
                x = get(c0)
                m = jnp.sum(x, axis=0, keepdims=True) * (1.0 / D)
                xc = x - m
                v = jnp.sum(xc * xc, axis=0, keepdims=True) * (1.0 / D)
                return xc * lax.rsqrt(v + 1e-5)
            for c0 in range(0, HT, LNC):
                n1 = norm(c0); n2 = norm(HT + c0)
                a11 = n1[0:256]; a12 = n1[256:512]; a21 = n2[0:256]; a22 = n2[256:512]
                for j, val in enumerate([a11 + a22, a21 + a22, a11, a22, a11 + a12, a21 - a11, a12 - a22]):
                    dst7[j, rs(c0, LNC), :] = pk(val.astype(BF16).T)
                dst_tail[c0:c0+LNC, 0:64] = n1[512:576].astype(BF16).T
                dst_tail[HT+c0:HT+c0+LNC, 0:64] = n2[512:576].astype(BF16).T

        def ln_f(pf, tie=None):
            def get(c0):
                x = xs[pf, :, c0:c0+LNC]
                if tie is not None:
                    x = jnp.concatenate([jnp.where(never, tie, x[0:8]), x[8:]], axis=0)
                return x
            ln_blocks(get, sa, xnf)

        def ln_a2(pa, xin, use_in, dst7, dst_tail):
            def first(c0):
                if use_in is True:
                    x = xin[:, c0:c0+LNC].astype(F32)
                else:
                    x = jnp.where(use_in, xin[:, c0:c0+LNC].astype(F32), xs[pa, :, c0:c0+LNC])
                xs[pa, :, c0:c0+LNC] = x
                return x
            ln_blocks(first, dst7, dst_tail)

        def halves(x):
            w = pltpu.bitcast(x, jnp.uint32)
            return [pltpu.unpack_elementwise(w, index=i, packed_dtype=BF16, unpacked_dtype=F32) for i in range(2)]

        def combos(p11, p12, p21, p22, signs):
            b = [halves(p) for p in (p11, p12, p21, p22)]
            outs = []
            for (i, j, sg) in signs:
                vals = [b[i][e] + b[j][e] if sg > 0 else b[i][e] - b[j][e] for e in range(2)]
                outs.append(pltpu.bitcast(pltpu.pack_elementwise(vals, packed_dtype=BF16), jnp.uint32))
            return outs
        RHS_SUMS = [(0, 3, 1), (1, 3, -1), (2, 0, -1), (0, 1, 1), (2, 3, 1)]
        LHS_SUMS = [(0, 3, 1), (2, 3, 1), (0, 1, 1), (2, 0, -1), (1, 3, -1)]

        def qkv_prep():
            NH = 896
            for r in range(0, NH, PRB):
                r1 = slice(r, r + PRB); r2 = slice(NH + r, NH + r + PRB)
                outs = combos(wqt[r1, 0:256], wqt[r2, 0:256], wqt[r1, 256:512], wqt[r2, 256:512], RHS_SUMS)
                for j, val in enumerate(outs):
                    tq[j, rs(r, PRB), :] = val

        def qkv_matmul(src7, src_tail):
            NH = 896
            m1 = dnt(upk(src7[0]), upk(tq[0]))
            m2 = dnt(upk(src7[1]), wqt[0:NH, 0:256])
            m3 = dnt(upk(src7[2]), upk(tq[1]))
            m4 = dnt(upk(src7[3]), upk(tq[2]))
            m5 = dnt(upk(src7[4]), wqt[NH:2*NH, 256:512])
            m6 = dnt(upk(src7[5]), upk(tq[3]))
            m7 = dnt(upk(src7[6]), upk(tq[4]))
            tl = dnt(src_tail[:, 0:64], wqt[:, 512:576])
            top = jnp.concatenate([m1 + m4 - m5 + m7, m3 + m5], axis=1)
            bot = jnp.concatenate([m2 + m4, m1 - m2 + m3 + m6], axis=1)
            return jnp.concatenate([top, bot], axis=0) + tl, [m1, m2, m3, m4, m5, m6, m7, tl][LT][0:8, 0:LNC]

        def wo_stage(pf):
            xs[pf] += lax.dot_general(wot[:, 0:D], os_[:, 0:D], NT, preferred_element_type=F32)

        def qkv_stage(pa, la, src, src_tail=None):
            for c in range(5):
                kb[pa, c, 0:HALO, :] = kt[la, c]
                vb[pa, c, 0:HALO, :] = vt[la, c]
            tie = None
            if QS: qkv, tie = qkv_matmul(src, src_tail)
            else: qkv = lax.dot_general(src[:, 0:D], wqt[:, 0:D], NT, preferred_element_type=F32)
            lane = lax.broadcasted_iota(jnp.int32, (TM, 128), 1)
            qs[pa, :, 0:512] = qkv[:, 0:512] * qscale
            t4 = qkv[:, 512:640]
            qs[pa, :, 512:640] = jnp.where(lane < 64, t4 * qscale, 0.0)
            for c in range(5):
                kk = qkv[:, 640+c*128:640+(c+1)*128] if c < 4 else pltpu.roll(t4, 64, 1)
                vv = qkv[:, 1152+c*128:1152+(c+1)*128]
                kb[pa, c, HALO:HALO+TM, :] = kk
                vb[pa, c, HALO:HALO+TM, :] = vv
                kt[la, c] = kk[TM-HALO:, :]
                vt[la, c] = vv[TM-HALO:, :]
            return tie

        def first_block_halo(pa):
            for c in range(5):
                kb[pa, c, 0:HALO, :] = jnp.zeros((HALO, 128), F32)
                vb[pa, c, 0:HALO, :] = jnp.broadcast_to(vb[pa, c, HALO:HALO+1, :], (HALO, 128))

        def att_tile(pa, r0, rt, mask_base):
            q = [qs[pa, pl.ds(r0, rt), c*128:(c+1)*128] for c in range(5)]
            lg = []
            for w in range(NW):
                acc = None
                for c in range(5):
                    kk = kb[pa, c, pl.ds(r0 + HALO - DIL*w, rt), :]
                    p = q[c] * kk
                    acc = p if acc is None else acc + p
                acc = acc + pltpu.roll(acc, 64, 1)
                acc = acc + pltpu.roll(acc, 32, 1)
                if mask_base is not None and w > 0:
                    pos = mask_base + lax.broadcasted_iota(jnp.int32, (rt, 128), 0)
                    acc = jnp.where(pos >= DIL*w, acc, -1e9 * LOG2E)
                lg.append(acc)
            mx = lg[0]
            for w in range(1, NW): mx = jnp.maximum(mx, lg[w])
            e = [jnp.exp2(a - mx) for a in lg]
            sm = e[0]
            for w in range(1, NW): sm = sm + e[w]
            inv = 1.0 / sm
            res = []
            for c in range(5):
                acc = None
                for w in range(NW):
                    vv = vb[pa, c, pl.ds(r0 + HALO - DIL*w, rt), :]
                    t = e[w] * vv
                    acc = t if acc is None else acc + t
                o = (acc * inv).astype(BF16)
                os_[pl.ds(r0, rt), c*128:(c+1)*128] = o
                res.append(o)
            return res

        def att_rows(pa, base, n, rt, pos0):
            if 'noatt' in ablate: return
            att_tile(pa, base, HALO, pos0)
            r = HALO
            while r < n:
                t = min(rt, n - r)
                att_tile(pa, base + r, t, None)
                r += t

        def pk(x):
            return pltpu.bitcast(x, jnp.uint32) if U32 else x
        def upk(x):
            return pltpu.bitcast(x, BF16) if U32 else x
        def rs(r0, n):
            return slice(r0 // 2, (r0 + n) // 2) if U32 else slice(r0, r0 + n)
        def ra(n):
            return slice(0, n // 2) if U32 else slice(0, n)

        def dot(a, b): return jnp.dot(a, b, preferred_element_type=F32)
        def dnt(a, b): return lax.dot_general(a, b, NT, preferred_element_type=F32)

        def ffn_prep_gu(f, k1, k2, ko):
            for w, t in ((wg, tg), (wu, tu)):
                for r in range(0, 256, PRB):
                    r1 = slice(r, r + PRB); r2 = slice(256 + r, 256 + r + PRB)
                    outs = combos(w[f, r1, k1], w[f, r1, k2], w[f, r2, k1], w[f, r2, k2], RHS_SUMS)
                    for j, val in enumerate(outs):
                        t[f, j, rs(r, PRB), ko] = val

        def ffn_prep_d(f, k1, k2, ko):
            for r in range(0, 288, PRB):
                n = min(PRB, 288 - r)
                r1 = slice(r, r + n); r2 = slice(288 + r, 288 + r + n)
                outs = combos(wd[f, r1, k1], wd[f, r1, k2], wd[f, r2, k1], wd[f, r2, k2], LHS_SUMS)
                for j, val in enumerate(outs):
                    td[f, j, rs(r, n), ko] = val

        def ffn_prep_inline(f):
            cp_g(f).wait(); cp_u(f).wait(); cp_d(f).wait()
            for c in range(FC // 256):
                gi = c // (fs // 128); cc = c % (fs // 128)
                ffn_prep_gu(f, slice(gi * GS + cc * 128, gi * GS + (cc + 1) * 128),
                           slice(gi * GS + fs + cc * 128, gi * GS + fs + (cc + 1) * 128), slice(c * 128, (c + 1) * 128))
                ffn_prep_d(f, slice(gi * GS + cc * 128, gi * GS + (cc + 1) * 128),
                           slice(gi * GS + fs + cc * 128, gi * GS + fs + (cc + 1) * 128), slice(c * 128, (c + 1) * 128))

        def ffn_prep(f):
            def dbody(c, _):
                gi = c // (fs // 128); cc = c % (fs // 128)
                k1 = pl.ds(pl.multiple_of(gi * GS + cc * 128, 128), 128)
                k2 = pl.ds(pl.multiple_of(gi * GS + fs + cc * 128, 128), 128)
                ko = pl.ds(pl.multiple_of(c * 128, 128), 128)
                ffn_prep_d(f, k1, k2, ko)
                q = c // (fs // 256); qq = c % (fs // 256)
                j1 = pl.ds(pl.multiple_of(q * fs + qq * 128, 128), 128)
                j2 = pl.ds(pl.multiple_of(q * fs + fs // 2 + qq * 128, 128), 128)
                ffn_prep_gu(f, j1, j2, ko)
                return 0
            lax.fori_loop(0, FC // 256, dbody, 0)

        def ffn_up(f, gi):
            tl = xnf[:, 0:64]
            hh = fs // 2
            def proj(w, t, kh):
                c0 = gi * GS + kh * fs
                k1 = slice(c0, c0 + hh); k2 = slice(c0 + hh, c0 + fs)
                ko = slice(c0 // 2, c0 // 2 + hh)
                m1 = dot(upk(sa[0]), upk(t[f, 0, :, ko]))
                m2 = dot(upk(sa[1]), w[f, 0:256, k1])
                m3 = dot(upk(sa[2]), upk(t[f, 1, :, ko]))
                m4 = dot(upk(sa[3]), upk(t[f, 2, :, ko]))
                m5 = dot(upk(sa[4]), w[f, 256:512, k2])
                m6 = dot(upk(sa[5]), upk(t[f, 3, :, ko]))
                m7 = dot(upk(sa[6]), upk(t[f, 4, :, ko]))
                tt = dot(tl, w[f, 512:576, c0:c0+fs])
                top = jnp.concatenate([m1 + m4 - m5 + m7, m3 + m5], axis=1) + tt[0:HT]
                bot = jnp.concatenate([m2 + m4, m1 - m2 + m3 + m6], axis=1) + tt[HT:TM]
                return top, bot
            hs = {}
            for kh in range(2):
                g = proj(wg, tg, kh); u = proj(wu, tu, kh)
                hs[(0, kh)] = _gelu(g[0]) * u[0]
                hs[(1, kh)] = _gelu(g[1]) * u[1]
            h11, h12, h21, h22 = hs[(0, 0)], hs[(0, 1)], hs[(1, 0)], hs[(1, 1)]
            b11, b12, b21, b22 = h11, h21, h12, h22
            return [v.astype(BF16) for v in (b11 + b22, b11, b12 - b22, b21 - b11, b22, b11 + b12, b21 + b22)]

        def ffn_down(pf, f, gi, hb):
            ko = slice(gi * fs, (gi + 1) * fs)
            k1 = slice(gi * GS, gi * GS + fs); k2 = slice(gi * GS + fs, (gi + 1) * GS)
            n1 = dnt(upk(td[f, 0, :, ko]), hb[0])
            n2 = dnt(upk(td[f, 1, :, ko]), hb[1])
            n3 = dnt(wd[f, 0:288, k1], hb[2])
            n4 = dnt(wd[f, 288:576, k2], hb[3])
            n5 = dnt(upk(td[f, 2, :, ko]), hb[4])
            n6 = dnt(upk(td[f, 3, :, ko]), hb[5])
            n7 = dnt(upk(td[f, 4, :, ko]), hb[6])
            xs[pf, 0:288, 0:HT] += n1 + n4 - n5 + n7
            xs[pf, 0:288, HT:TM] += n3 + n5
            xs[pf, 288:576, 0:HT] += n2 + n4
            xs[pf, 288:576, HT:TM] += n1 - n2 + n3 + n6

        def ffn_chunk(pf, f, att_parts):
            prev = None
            for gi in range(NG):
                cur = ffn_up(f, gi)
                outs = att_parts[gi]()
                if TIE and outs:
                    z = cur[1][0:RT, 0:128]
                    for o in outs: z = jnp.where(never, o, z)
                    top = jnp.concatenate([z, cur[1][0:RT, 128:]], axis=1) if fs > 128 else z
                    cur[1] = jnp.concatenate([top, cur[1][RT:]], axis=0)
                if prev is not None: ffn_down(pf, f, gi - 1, prev)
                prev = cur
            ffn_down(pf, f, NG - 1, prev)

        @pl.when(s == 0)
        def _():
            flag[0] = 0
        never = flag[0] != 0
        pa = s % 2
        pf = 1 - pa
        la = (s // 2) % 2
        ab = blk_of(s)

        @pl.when(s == 0)
        @jax.named_scope("P0")
        def _():
            prep()
            if QS: qkv_prep()
            if QS:
                qkv_stage(0, 0, sq, xqt)
                ln_a2(1, xin.at[1], True, sa, xnf)
            else:
                qkv_stage(0, 0, xna)
                ln_a(1, xin.at[1], True, xn1)
            first_block_halo(0)
            prep_wo()

        @pl.when(s == 0)
        @jax.named_scope("P1")
        def _():
            if PP >= 1: ffn_prep_inline(0)
            if 'attlast' in ablate:
                (qkv_stage(1, 0, sa, xnf) if QS else qkv_stage(1, 0, xn1))
                att_rows(0, 0, TM, RTP, 0)
            else:
                att_rows(0, 0, TM, RTP, 0)
                (qkv_stage(1, 0, sa, xnf) if QS else qkv_stage(1, 0, xn1))

        for b in range(2, NB):
            @pl.when(s == 4 * (b // 2) + b % 2)
            def _():
                cp_x(b).wait()

        @pl.when(jnp.logical_and(s > 1, s < NSLOT - 1))
        @jax.named_scope("R")
        def _():
            if QS: ln_a2(pa, xin.at[jnp.minimum(ab, NB - 1)], la == 0, sq, xqt)
            else: ln_a(pa, xin.at[jnp.minimum(ab, NB - 1)], la == 0, xna)
            wo_stage(pf)
            tie = (qkv_stage(pa, la, sq, xqt) if QS else qkv_stage(pa, la, xna))
            ln_f(pf, tie if LT >= 0 else None)

        if PP >= 2:
            @pl.when(s == 1)
            @jax.named_scope("RS1")
            def _():
                ffn_prep_inline(1)
                wo_stage(pf)
                ln_f(pf)

        @pl.when(jnp.logical_or(s == 1, s == NSLOT - 1) if PP < 2 else s == NSLOT - 1)
        @jax.named_scope("RS")
        def _():
            wo_stage(pf)
            ln_f(pf)

        @pl.when(s == 2)
        def _():
            first_block_halo(0)

        @pl.when(s > 0)
        @jax.named_scope("LOOP")
        def _():
            def body(f, _):
                @pl.when(s == 1)
                def _():
                    for ff in range(PP, NF):
                        @pl.when(f == ff)
                        def _():
                            cp_g(ff).wait(); cp_u(ff).wait(); cp_d(ff).wait()
                    @pl.when(f >= PP)
                    def _():
                        ffn_prep(f)
                base = pl.multiple_of(jnp.minimum(f * PR, TM - PR), PRQ)
                tiles = [functools.partial(att_tile, pa, base + r, min(RT, PR - r), (ab * TM + base) if r == 0 else None)
                         for r in range(0, PR, RT)]
                nper = -(-len(tiles) // NG)
                def part(j):
                    def run():
                        if 'noatt' in ablate: return []
                        return [o for t in tiles[j*nper:(j+1)*nper] for o in t()]
                    return run
                ffn_chunk(pf, f, [part(j) for j in range(NG)])
                return 0
            lax.fori_loop(0, NF, body, 0)

        @pl.when(jnp.logical_and(s > 0, ((s - 1) // 2) % 2 == 1))
        def _():
            o_ref[...] = xs[pf].astype(o_ref.dtype)

    def x_map(s):
        la = (s // 2) % 2
        b = jnp.where(la == 0, blk_of(s), 2 * (s // 4) + 1)
        return (0, jnp.clip(b, 0, NB - 1))

    def o_map(s):
        fidx = jnp.maximum(s - 1, 0)
        b = 2 * (fidx // 4) + jnp.where(fidx % 4 == 3, 1, 0)
        return (0, b)

    def fn(A_x, A_wqkv, A_wo, B_x, B_w_gate, B_w_up, B_w_down):
        xT = A_x.reshape(S, D).T
        out = pl.pallas_call(
            kernel,
            grid=(NSLOT,),
            in_specs=[pl.BlockSpec(memory_space=pltpu.HBM)] * 6,
            out_specs=pl.BlockSpec((D, TM), o_map),
            out_shape=jax.ShapeDtypeStruct((D, S), BF16),
            scratch_shapes=[
                pltpu.VMEM((NB, D, TM), BF16), pltpu.VMEM((D, 3 * D), BF16), pltpu.VMEM((D, D), BF16),
                pltpu.VMEM((5, 1792, 128), F32),
                pltpu.VMEM((1792, 640), BF16), pltpu.VMEM((D, 640), BF16),
                pltpu.VMEM((NF, D, FC), BF16), pltpu.VMEM((NF, D, FC), BF16), pltpu.VMEM((NF, D, FC), BF16),
                pltpu.VMEM((NF, 5, 128, FC // 2), jnp.uint32), pltpu.VMEM((NF, 5, 128, FC // 2), jnp.uint32),
                pltpu.VMEM((NF, 5, 144, FC // 2), jnp.uint32) if U32 else pltpu.VMEM((NF, 5, 288, FC // 2), BF16),
                pltpu.VMEM((2, D, TM), F32), pltpu.VMEM((TM, 640), BF16), pltpu.VMEM((TM, 640), BF16), pltpu.VMEM((TM, 128), BF16), pltpu.VMEM((7, HT // 2, 256), jnp.uint32) if U32 else pltpu.VMEM((7, HT, 256), BF16),
                pltpu.VMEM((7, HT // 2, 256), jnp.uint32) if U32 else pltpu.VMEM((7, HT, 256), BF16),
                pltpu.VMEM((TM, 128), BF16),
                pltpu.VMEM((5, 448, 256), jnp.uint32) if U32 else pltpu.VMEM((5, 896, 256), BF16),
                pltpu.VMEM((2, TM, 640), F32),
                pltpu.VMEM((2, 5, TM + HALO + KPAD, 128), F32), pltpu.VMEM((2, 5, TM + HALO + KPAD, 128), F32),
                pltpu.VMEM((2, 5, HALO, 128), F32), pltpu.VMEM((2, 5, HALO, 128), F32),
                pltpu.VMEM((TM, 640), BF16),
                pltpu.SemaphoreType.DMA((2 + 3 * NF,)), pltpu.SemaphoreType.DMA((5 + NB,)), pltpu.SMEM((1,), jnp.int32),
            ],
            compiler_params=pltpu.CompilerParams(dimension_semantics=("arbitrary",), vmem_limit_bytes=112 * 1024 * 1024, flags=({FLAG: True} if FLAG else None)),
        )(xT, A_wqkv, A_wo, B_w_gate, B_w_up, B_w_down.T)
        return out.T.reshape(1, S, D)
    return fn


_fn = make_kernel(ablate='attlast')


@jax.jit
def pallas_interleave_layers__sliding_local_dilated__glu_gated_geglu__prompt_kernel(
    A_x: jax.Array,
    A_wqkv: jax.Array,
    A_wo: jax.Array,
    B_x: jax.Array,
    B_w_gate: jax.Array,
    B_w_up: jax.Array,
    B_w_down: jax.Array,
):
    return _fn(A_x, A_wqkv, A_wo, B_x, B_w_gate, B_w_up, B_w_down)
```

```python
import numpy as np
import jax
import jax.numpy as jnp
from jax import lax
import jax.experimental.pallas as pl
import jax.experimental.pallas.tpu as pltpu

S, D, F, H, DH = 2048, 576, 4608, 32, 18
NW, DIL = 8, 2
HALO = 16
KPAD = 16
TM, HT = 512, 256
NB = S // TM
NSLOT = 2 * NB + 1
FC, GS = 1536, 512
NF, NG, FS, HH = F // FC, FC // GS, GS // 2, GS // 4
PR, RT, RTP = 192, 32, 128
LNC, PRB = 256, 32
NH = 896
LOG2E = 1.4426950408889634
NT = (((1,), (1,)), ((), ()))
F32, BF16, U32 = jnp.float32, jnp.bfloat16, jnp.uint32
RHS_SUMS = [(0, 3, 1), (1, 3, -1), (2, 0, -1), (0, 1, 1), (2, 3, 1)]
LHS_SUMS = [(0, 3, 1), (2, 3, 1), (0, 1, 1), (2, 0, -1), (1, 3, -1)]


def _gelu(g):
    c = np.float32(np.sqrt(2 / np.pi))
    inner = g * (c + (c * 0.044715) * (g * g))
    hg = 0.5 * g
    return hg + hg * jnp.tanh(inner)


def _pk(x):
    return pltpu.bitcast(x, U32)


def _upk(x):
    return pltpu.bitcast(x, BF16)


def _dot(a, b):
    return jnp.dot(a, b, preferred_element_type=F32)


def _dnt(a, b):
    return lax.dot_general(a, b, NT, preferred_element_type=F32)


def _sums(blocks, signs):
    b = [[pltpu.unpack_elementwise(_pk(p), index=i, packed_dtype=BF16, unpacked_dtype=F32) for i in range(2)]
         for p in blocks]
    outs = []
    for (i, j, sg) in signs:
        vals = [b[i][e] + b[j][e] if sg > 0 else b[i][e] - b[j][e] for e in range(2)]
        outs.append(pltpu.bitcast(pltpu.pack_elementwise(vals, packed_dtype=BF16), U32))
    return outs


def _blk_of(a):
    return 2 * (a // 4) + a % 2


def _kernel(x_hbm, wqkv_hbm, wo_hbm, wg_hbm, wu_hbm, wd_hbm, o_ref,
            xin, wraw, woraw, t32, wqt, wot, wg, wu, wd, tg, tu, td, xs, xnf, sa, sq, xqt, tq,
            qs, kb, vb, kt, vt, os_, sems, sems2):
    s = pl.program_id(0)
    qscale = (DH ** -0.5) * LOG2E

    def cp_qkv(c):
        n = 128 if c < 4 else 64
        return pltpu.make_async_copy(wqkv_hbm.at[pl.ds(c * 128, n), :], wraw.at[pl.ds(c * 128, n), :], sems2.at[c])
    def cp_x(b): return pltpu.make_async_copy(x_hbm.at[:, pl.ds(b * TM, TM)], xin.at[b], sems2.at[5 + b])
    def cp_o(): return pltpu.make_async_copy(wo_hbm, woraw, sems.at[0])
    def cp_g(f): return pltpu.make_async_copy(wg_hbm.at[:, pl.ds(f * FC, FC)], wg.at[f], sems.at[1 + 3 * f])
    def cp_u(f): return pltpu.make_async_copy(wu_hbm.at[:, pl.ds(f * FC, FC)], wu.at[f], sems.at[2 + 3 * f])
    def cp_d(f): return pltpu.make_async_copy(wd_hbm.at[:, pl.ds(f * FC, FC)], wd.at[f], sems.at[3 + 3 * f])

    def ln_blocks(get, dst7, dst_tail):
        def norm(c0):
            x = get(c0)
            m = jnp.sum(x, axis=0, keepdims=True) * (1.0 / D)
            xc = x - m
            v = jnp.sum(xc * xc, axis=0, keepdims=True) * (1.0 / D)
            return xc * lax.rsqrt(v + 1e-5)
        for c0 in range(0, HT, LNC):
            n1 = norm(c0); n2 = norm(HT + c0)
            a11 = n1[0:256]; a12 = n1[256:512]; a21 = n2[0:256]; a22 = n2[256:512]
            for j, val in enumerate([a11 + a22, a21 + a22, a11, a22, a11 + a12, a21 - a11, a12 - a22]):
                dst7[j, c0 // 2:(c0 + LNC) // 2, :] = _pk(val.astype(BF16).T)
            dst_tail[c0:c0 + LNC, 0:64] = n1[512:576].astype(BF16).T
            dst_tail[HT + c0:HT + c0 + LNC, 0:64] = n2[512:576].astype(BF16).T

    def ln_f(pf):
        ln_blocks(lambda c0: xs[pf, :, c0:c0 + LNC], sa, xnf)

    def ln_a(pa, x16, use_in, dst7, dst_tail):
        def get(c0):
            x = x16[:, c0:c0 + LNC].astype(F32)
            if use_in is not True:
                x = jnp.where(use_in, x, xs[pa, :, c0:c0 + LNC])
            xs[pa, :, c0:c0 + LNC] = x
            return x
        ln_blocks(get, dst7, dst_tail)

    def prep():
        cp_x(0).start()
        for c in range(5): cp_qkv(c).start()
        cp_x(1).start(); cp_o().start()
        kt[...] = jnp.zeros(kt.shape, F32)
        vt[...] = jnp.zeros(vt.shape, F32)
        wqt[1728:1792, :] = jnp.zeros((64, 640), BF16)
        cp_x(0).wait()
        ln_a(0, xin.at[0], True, sq, xqt)
        def dest(p, d):
            if p == 0: return d * 32
            if p == 1: return 576 + (d - 16) * 32 if d >= 16 else 640 + d * 32
            return 1152 + d * 32
        for c in range(5):
            cp_qkv(c).wait()
            kw = 128 if c < 4 else 64
            for j in range(14):
                nw = 128 if j < 13 else 64
                blk = wraw[c * 128:c * 128 + kw, j * 128:j * 128 + nw].astype(F32)
                if kw < 128: blk = jnp.concatenate([blk, jnp.zeros((128 - kw, nw), F32)], axis=0)
                if nw < 128: blk = jnp.concatenate([blk, jnp.zeros((128, 128 - nw), F32)], axis=1)
                t32[c, j * 128:(j + 1) * 128, :] = blk.T
            for p in range(3):
                for d in range(DH):
                    rows = t32[c, pl.ds(p * D + d, H, stride=DH), :]
                    r0 = dest(p, d)
                    wqt[r0:r0 + H, c * 128:(c + 1) * 128] = rows.astype(BF16)
        cp_x(1).wait()
        for f in range(NF):
            cp_g(f).start(); cp_u(f).start(); cp_d(f).start()
        for b in range(2, NB): cp_x(b).start()

    def prep_wo():
        cp_o().wait()
        for c in range(5):
            nw = 128 if c < 4 else 64
            blk = woraw[:, c * 128:c * 128 + nw].astype(F32)
            if nw < 128: blk = jnp.concatenate([blk, jnp.zeros((D, 128 - nw), F32)], axis=1)
            t32[c, 0:D, :] = blk
        for c in range(5):
            parts = [t32[c, pl.ds(d, H, stride=DH), :] for d in range(DH)] + [jnp.zeros((64, 128), F32)]
            res = jnp.concatenate(parts, axis=0).T.astype(BF16)
            nw = 128 if c < 4 else 64
            wot[c * 128:c * 128 + nw, :] = res[:nw]

    def qkv_prep():
        for r in range(0, NH, PRB):
            r1 = slice(r, r + PRB); r2 = slice(NH + r, NH + r + PRB)
            outs = _sums((wqt[r1, 0:256], wqt[r2, 0:256], wqt[r1, 256:512], wqt[r2, 256:512]), RHS_SUMS)
            for j, val in enumerate(outs):
                tq[j, r // 2:(r + PRB) // 2, :] = val

    def ffn_prep(f):
        def body(c, _):
            al = lambda v: pl.ds(pl.multiple_of(v, 128), 128)
            gi = c // (FS // 128); cc = c % (FS // 128)
            k1, k2, ko = al(gi * GS + cc * 128), al(gi * GS + FS + cc * 128), al(c * 128)
            for r in range(0, 288, PRB):
                r1 = slice(r, r + PRB); r2 = slice(288 + r, 288 + r + PRB)
                outs = _sums((wd[f, r1, k1], wd[f, r1, k2], wd[f, r2, k1], wd[f, r2, k2]), LHS_SUMS)
                for j, val in enumerate(outs):
                    td[f, j, r // 2:(r + PRB) // 2, ko] = val
            q = c // (FS // 256); qq = c % (FS // 256)
            j1, j2 = al(q * FS + qq * 128), al(q * FS + HH + qq * 128)
            for w, t in ((wg, tg), (wu, tu)):
                for r in range(0, 256, PRB):
                    r1 = slice(r, r + PRB); r2 = slice(256 + r, 256 + r + PRB)
                    outs = _sums((w[f, r1, j1], w[f, r1, j2], w[f, r2, j1], w[f, r2, j2]), RHS_SUMS)
                    for j, val in enumerate(outs):
                        t[f, j, r // 2:(r + PRB) // 2, ko] = val
            return 0
        lax.fori_loop(0, FC // 256, body, 0, unroll=True)

    def wo_stage(pf):
        xs[pf] += _dnt(wot[:, 0:D], os_[:, 0:D])

    def qkv_stage(pa, la, src7, src_tail):
        for c in range(5):
            kb[pa, c, 0:HALO, :] = kt[la, c]
            vb[pa, c, 0:HALO, :] = vt[la, c]
        m1 = _dnt(_upk(src7[0]), _upk(tq[0]))
        m2 = _dnt(_upk(src7[1]), wqt[0:NH, 0:256])
        m3 = _dnt(_upk(src7[2]), _upk(tq[1]))
        m4 = _dnt(_upk(src7[3]), _upk(tq[2]))
        m5 = _dnt(_upk(src7[4]), wqt[NH:2 * NH, 256:512])
        m6 = _dnt(_upk(src7[5]), _upk(tq[3]))
        m7 = _dnt(_upk(src7[6]), _upk(tq[4]))
        tl = _dnt(src_tail[:, 0:64], wqt[:, 512:576])
        top = jnp.concatenate([m1 + m4 - m5 + m7, m3 + m5], axis=1)
        bot = jnp.concatenate([m2 + m4, m1 - m2 + m3 + m6], axis=1)
        qkv = jnp.concatenate([top, bot], axis=0) + tl
        lane = lax.broadcasted_iota(jnp.int32, (TM, 128), 1)
        qs[pa, :, 0:512] = qkv[:, 0:512] * qscale
        t4 = qkv[:, 512:640]
        qs[pa, :, 512:640] = jnp.where(lane < 64, t4 * qscale, 0.0)
        for c in range(5):
            kk = qkv[:, 640 + c * 128:640 + (c + 1) * 128] if c < 4 else pltpu.roll(t4, 64, 1)
            vv = qkv[:, 1152 + c * 128:1152 + (c + 1) * 128]
            kb[pa, c, HALO:HALO + TM, :] = kk
            vb[pa, c, HALO:HALO + TM, :] = vv
            kt[la, c] = kk[TM - HALO:, :]
            vt[la, c] = vv[TM - HALO:, :]

    def first_block_halo(pa):
        for c in range(5):
            kb[pa, c, 0:HALO, :] = jnp.zeros((HALO, 128), F32)
            vb[pa, c, 0:HALO, :] = jnp.broadcast_to(vb[pa, c, HALO:HALO + 1, :], (HALO, 128))

    def att_tile(pa, r0, rt, pos0):
        q = [qs[pa, pl.ds(r0, rt), c * 128:(c + 1) * 128] for c in range(5)]
        lg = []
        for w in range(NW):
            acc = None
            for c in range(5):
                p = q[c] * kb[pa, c, pl.ds(r0 + HALO - DIL * w, rt), :]
                acc = p if acc is None else acc + p
            acc = acc + pltpu.roll(acc, 64, 1)
            acc = acc + pltpu.roll(acc, 32, 1)
            if pos0 is not None and w > 0:
                pos = pos0 + lax.broadcasted_iota(jnp.int32, (rt, 128), 0)
                acc = jnp.where(pos >= DIL * w, acc, -1e9 * LOG2E)
            lg.append(acc)
        mx = lg[0]
        for w in range(1, NW): mx = jnp.maximum(mx, lg[w])
        e = [jnp.exp2(a - mx) for a in lg]
        sm = e[0]
        for w in range(1, NW): sm = sm + e[w]
        inv = 1.0 / sm
        for c in range(5):
            acc = None
            for w in range(NW):
                t = e[w] * vb[pa, c, pl.ds(r0 + HALO - DIL * w, rt), :]
                acc = t if acc is None else acc + t
            os_[pl.ds(r0, rt), c * 128:(c + 1) * 128] = (acc * inv).astype(BF16)

    def ffn_up(f, gi):
        tl = xnf[:, 0:64]
        def proj(w, t, kh):
            c0 = gi * GS + kh * FS
            k1 = slice(c0, c0 + HH); k2 = slice(c0 + HH, c0 + FS); ko = slice(c0 // 2, c0 // 2 + HH)
            m1 = _dot(_upk(sa[0]), _upk(t[f, 0, :, ko]))
            m2 = _dot(_upk(sa[1]), w[f, 0:256, k1])
            m3 = _dot(_upk(sa[2]), _upk(t[f, 1, :, ko]))
            m4 = _dot(_upk(sa[3]), _upk(t[f, 2, :, ko]))
            m5 = _dot(_upk(sa[4]), w[f, 256:512, k2])
            m6 = _dot(_upk(sa[5]), _upk(t[f, 3, :, ko]))
            m7 = _dot(_upk(sa[6]), _upk(t[f, 4, :, ko]))
            tt = _dot(tl, w[f, 512:576, c0:c0 + FS])
            top = jnp.concatenate([m1 + m4 - m5 + m7, m3 + m5], axis=1) + tt[0:HT]
            bot = jnp.concatenate([m2 + m4, m1 - m2 + m3 + m6], axis=1) + tt[HT:TM]
            return top, bot
        hs = {}
        for kh in range(2):
            g = proj(wg, tg, kh); u = proj(wu, tu, kh)
            hs[(0, kh)] = _gelu(g[0]) * u[0]
            hs[(1, kh)] = _gelu(g[1]) * u[1]
        b11, b12, b21, b22 = hs[(0, 0)], hs[(1, 0)], hs[(0, 1)], hs[(1, 1)]
        return [v.astype(BF16) for v in (b11 + b22, b11, b12 - b22, b21 - b11, b22, b11 + b12, b21 + b22)]

    def ffn_down(pf, f, gi, hb):
        ko = slice(gi * FS, (gi + 1) * FS)
        k1 = slice(gi * GS, gi * GS + FS); k2 = slice(gi * GS + FS, (gi + 1) * GS)
        n1 = _dnt(_upk(td[f, 0, :, ko]), hb[0])
        n2 = _dnt(_upk(td[f, 1, :, ko]), hb[1])
        n3 = _dnt(wd[f, 0:288, k1], hb[2])
        n4 = _dnt(wd[f, 288:576, k2], hb[3])
        n5 = _dnt(_upk(td[f, 2, :, ko]), hb[4])
        n6 = _dnt(_upk(td[f, 3, :, ko]), hb[5])
        n7 = _dnt(_upk(td[f, 4, :, ko]), hb[6])
        xs[pf, 0:288, 0:HT] += n1 + n4 - n5 + n7
        xs[pf, 0:288, HT:TM] += n3 + n5
        xs[pf, 288:576, 0:HT] += n2 + n4
        xs[pf, 288:576, HT:TM] += n1 - n2 + n3 + n6

    def ffn_chunk(pf, f):
        prev = None
        for gi in range(NG):
            cur = ffn_up(f, gi)
            if prev is not None: ffn_down(pf, f, gi - 1, prev)
            prev = cur
        ffn_down(pf, f, NG - 1, prev)

    pa = s % 2
    pf = 1 - pa
    la = (s // 2) % 2
    ab = _blk_of(s)

    @pl.when(s == 0)
    def _():
        prep()
        qkv_prep()
        qkv_stage(0, 0, sq, xqt)
        ln_a(1, xin.at[1], True, sa, xnf)
        prep_wo()
        first_block_halo(0)

    @pl.when(s == 0)
    def _():
        qkv_stage(1, 0, sa, xnf)
        att_tile(0, 0, HALO, 0)
        r = HALO
        while r < TM:
            t = min(RTP, TM - r)
            att_tile(0, r, t, None)
            r += t

    for b in range(2, NB):
        @pl.when(s == 4 * (b // 2) + b % 2)
        def _():
            cp_x(b).wait()

    @pl.when(jnp.logical_and(s > 1, s < NSLOT - 1))
    def _():
        ln_a(pa, xin.at[jnp.minimum(ab, NB - 1)], la == 0, sq, xqt)
        wo_stage(pf)
        ln_f(pf)
        qkv_stage(pa, la, sq, xqt)

    @pl.when(jnp.logical_or(s == 1, s == NSLOT - 1))
    def _():
        wo_stage(pf)
        ln_f(pf)

    @pl.when(s == 2)
    def _():
        first_block_halo(0)

    @pl.when(s > 0)
    def _():
        def body(f, _):
            @pl.when(s == 1)
            def _():
                for ff in range(NF):
                    @pl.when(f == ff)
                    def _():
                        cp_g(ff).wait(); cp_u(ff).wait(); cp_d(ff).wait()
                ffn_prep(f)
            ffn_chunk(pf, f)
            base = pl.multiple_of(jnp.minimum(f * PR, TM - PR), RT)
            for r in range(0, PR, RT):
                att_tile(pa, base + r, RT, (ab * TM + base) if r == 0 else None)
            return 0
        lax.fori_loop(0, NF, body, 0)

    @pl.when(jnp.logical_and(s > 0, ((s - 1) // 2) % 2 == 1))
    def _():
        o_ref[...] = xs[pf].astype(o_ref.dtype)


def _o_map(s):
    fidx = jnp.maximum(s - 1, 0)
    return (0, 2 * (fidx // 4) + jnp.where(fidx % 4 == 3, 1, 0))


@jax.jit
def pallas_interleave_layers__sliding_local_dilated__glu_gated_geglu__prompt_kernel(
    A_x: jax.Array,
    A_wqkv: jax.Array,
    A_wo: jax.Array,
    B_x: jax.Array,
    B_w_gate: jax.Array,
    B_w_up: jax.Array,
    B_w_down: jax.Array,
):
    vm = pltpu.VMEM
    out = pl.pallas_call(
        _kernel,
        grid=(NSLOT,),
        in_specs=[pl.BlockSpec(memory_space=pltpu.HBM)] * 6,
        out_specs=pl.BlockSpec((D, TM), _o_map),
        out_shape=jax.ShapeDtypeStruct((D, S), BF16),
        scratch_shapes=[
            vm((NB, D, TM), BF16), vm((D, 3 * D), BF16), vm((D, D), BF16), vm((5, 1792, 128), F32),
            vm((1792, 640), BF16), vm((D, 640), BF16),
            vm((NF, D, FC), BF16), vm((NF, D, FC), BF16), vm((NF, D, FC), BF16),
            vm((NF, 5, 128, FC // 2), U32), vm((NF, 5, 128, FC // 2), U32), vm((NF, 5, 144, FC // 2), U32),
            vm((2, D, TM), F32), vm((TM, 128), BF16), vm((7, HT // 2, 256), U32), vm((7, HT // 2, 256), U32),
            vm((TM, 128), BF16), vm((5, NH // 2, 256), U32),
            vm((2, TM, 640), F32),
            vm((2, 5, TM + HALO + KPAD, 128), F32), vm((2, 5, TM + HALO + KPAD, 128), F32),
            vm((2, 5, HALO, 128), F32), vm((2, 5, HALO, 128), F32),
            vm((TM, 640), BF16),
            pltpu.SemaphoreType.DMA((1 + 3 * NF,)), pltpu.SemaphoreType.DMA((5 + NB,)),
        ],
        compiler_params=pltpu.CompilerParams(
            dimension_semantics=("arbitrary",), vmem_limit_bytes=112 * 1024 * 1024,
            flags={"XLA_TPU_EVENLY_DISTRIBUTE_CRITICAL_NODES": True}),
    )(A_x.reshape(S, D).T, A_wqkv, A_wo, B_w_gate, B_w_up, B_w_down.T)
    return out.T.reshape(1, S, D)
```
